```python
import jax
import jax.numpy as jnp

def _softmax(x, axis=-1):
    return jax.nn.softmax(x, axis=axis)

def _gelu(x):
    return jax.nn.gelu(x, approximate=True)

def _silu(x):
    return jax.nn.silu(x)

def _sigmoid(x):
    return jax.nn.sigmoid(x)

def _layernorm(x, axis=-1, eps=1e-05):
    m = jnp.mean(x, axis=axis, keepdims=True)
    v = jnp.var(x, axis=axis, keepdims=True)
    return (x - m) / jnp.sqrt(v + eps)

def _scatter_add(tgt, idx, src, axis=0):
    return tgt.at[idx].add(src)

def _segment_sum(src, seg, n):
    return jax.ops.segment_sum(src, seg, n)

class _Rng:

    def __init__(self, key):
        self._k = key

    def _next(self):
        self._k, sub = jax.random.split(self._k)
        return sub

    def normal(self, shape):
        return jax.random.normal(self._next(), shape, dtype=jnp.bfloat16)

    def randint(self, lo, hi, shape):
        return jax.random.randint(self._next(), shape, lo, hi, dtype=jnp.int32)

    def uniform(self, shape, lo=0.0, hi=1.0):
        return jax.random.uniform(self._next(), shape, jnp.bfloat16, lo, hi)

    def permutation(self, n):
        return jax.random.permutation(self._next(), n)
kernel_name = 'interleave_layers__memory_aug_infini_attn__moe_arch_mod__prompt'

def setup_inputs():
    _rng = _Rng(jax.random.key(int.from_bytes(__import__("os").urandom(4), "little")))
    _w = lambda a: (lambda t: t.astype(jnp.bfloat16) if jnp.issubdtype(t.dtype, jnp.floating) else t)(jnp.asarray(a))

    def _A_setup():
        B, S, D, H = (1, 2048, 1024, 32)
        N = 4
        L = max(1, S // N)
        sc = D ** (-0.5)
        return {'x': _w((lambda *s: _rng.normal(s) * 0.05)(B, N * L, D)), 'wq': _w((lambda *s: _rng.normal(s) * 0.05)(D, D) * sc), 'wk': _w((lambda *s: _rng.normal(s) * 0.05)(D, D) * sc), 'wv': _w((lambda *s: _rng.normal(s) * 0.05)(D, D) * sc), 'wo': _w((lambda *s: _rng.normal(s) * 0.05)(D, D) * sc), 'beta': _w((lambda *s: _rng.normal(s) * 0.05)(H))}
    _A_in = _A_setup()

    def _B_setup():
        B, S, D, F, C = (1, 2048, 1024, 3584, 2)
        return {'x': _w((lambda *s: _rng.normal(s) * 0.05)(B, S, D)), 'w_r': _w((lambda *s: _rng.normal(s) * 0.05)(D)), 'w_gate': _w((lambda *s: _rng.normal(s) * 0.05)(D, F)), 'w_up': _w((lambda *s: _rng.normal(s) * 0.05)(D, F)), 'w_down': _w((lambda *s: _rng.normal(s) * 0.05)(F, D))}
    _B_in = _B_setup()
    return {'A_x': _A_in['x'], 'A_wq': _A_in['wq'], 'A_wk': _A_in['wk'], 'A_wv': _A_in['wv'], 'A_wo': _A_in['wo'], 'A_beta': _A_in['beta'], 'B_x': _B_in['x'], 'B_w_r': _B_in['w_r'], 'B_w_gate': _B_in['w_gate'], 'B_w_up': _B_in['w_up'], 'B_w_down': _B_in['w_down']}

def reference(A_x, A_wq, A_wk, A_wv, A_wo, A_beta, B_x, B_w_r, B_w_gate, B_w_up, B_w_down):

    def _A_ref(x, wq, wk, wv, wo, beta):
        B, S, D = x.shape
        H = 32
        Dh = D // H
        N = 4
        L = S // N
        q = (lambda x, *d: x.transpose(*d))((x @ wq).reshape(B, S, H, Dh), 0, 2, 1, 3).reshape(B, H, N, L, Dh)
        k = (lambda x, *d: x.transpose(*d))((x @ wk).reshape(B, S, H, Dh), 0, 2, 1, 3).reshape(B, H, N, L, Dh)
        v = (lambda x, *d: x.transpose(*d))((x @ wv).reshape(B, S, H, Dh), 0, 2, 1, 3).reshape(B, H, N, L, Dh)
        phi = lambda t: jnp.where(t > 0, t + 1.0, jnp.exp(t))
        scale = Dh ** (-0.5)
        ar = jnp.arange(L)
        mask = (lambda x, dt: x.astype(dt))(ar[:, None] < ar[None, :], x.dtype) * -1000000000.0
        g = _sigmoid(beta).reshape(1, H, 1, 1)
        M = jnp.einsum('bhd,bhe->bhde', q[:, :, 0, 0, :] * 0.0, q[:, :, 0, 0, :] * 0.0)
        z = q[:, :, 0, 0, :] * 0.0
        outs = []
        for s in range(N):
            qs, ks, vs = (q[:, :, s].copy(), k[:, :, s].copy(), v[:, :, s].copy())
            logits = jnp.einsum('bhqd,bhkd->bhqk', qs, ks) * scale + mask
            p = _softmax(logits, axis=-1)
            a_dot = jnp.einsum('bhqk,bhkd->bhqd', p, vs)
            pq = phi(qs)
            num = jnp.einsum('bhld,bhde->bhle', pq, M)
            den = jnp.einsum('bhld,bhd->bhl', pq, z)[..., None] + 1e-06
            a_mem = num / den
            o = g * a_mem + (1.0 - g) * a_dot
            outs.append(o)
            pk = phi(ks)
            M = M + jnp.einsum('bhld,bhle->bhde', pk, vs)
            z = z + jnp.einsum('bhld->bhd', pk)
        o = (lambda x, *d: x.transpose(*d))(jnp.stack(outs, 2).reshape(B, H, S, Dh), 0, 2, 1, 3).reshape(B, S, D)
        return o @ wo

    def _B_ref(x, w_r, w_gate, w_up, w_down):
        B, S, D = x.shape
        C = 2
        r = x @ w_r
        idx = jnp.argsort(-r, axis=-1)[:, :C]
        idx_e = jnp.repeat(idx.reshape(B, C, 1), D, axis=2)
        x_sel = jnp.take_along_axis(x, idx_e, axis=1)
        g = _silu(x_sel @ w_gate)
        u = x_sel @ w_up
        y = g * u @ w_down
        r_sel = _sigmoid(jnp.take_along_axis(r, idx, axis=1))
        y = y * r_sel.reshape(B, C, 1)
        b_off = (jnp.arange(B) * S).reshape(B, 1)
        flat_idx = (idx + b_off).reshape(B * C)
        zero = (x * 0.0).reshape(B * S, D)
        upd = _scatter_add(zero, flat_idx, y.reshape(B * C, D), axis=0)
        return x + upd.reshape(B, S, D)
    x = A_x
    x = x + _A_ref(_layernorm(x, axis=-1), A_wq, A_wk, A_wv, A_wo, A_beta)
    x = x + _B_ref(_layernorm(x, axis=-1), B_w_r, B_w_gate, B_w_up, B_w_down)
    x = x + _A_ref(_layernorm(x, axis=-1), A_wq, A_wk, A_wv, A_wo, A_beta)
    x = x + _B_ref(_layernorm(x, axis=-1), B_w_r, B_w_gate, B_w_up, B_w_down)
    return x
```

```python
import functools

import jax
import jax.numpy as jnp
import numpy as np
from jax import lax
import jax.experimental.pallas as pl
import jax.experimental.pallas.tpu as pltpu

S = 2048
D = 1024
NSEG = 4
L = S // NSEG
H = 32
DH = D // H
NG = 8
F = 3584
NF = F // 128
CH = L // NG
EPS = 1e-5
LOG2E = 1.4426950408889634
QSCALE = (DH ** -0.5) * LOG2E
NEG = -1e30

bf16 = jnp.bfloat16
f32 = jnp.float32
u32 = jnp.uint32
i32 = jnp.int32
NT = (((1,), (1,)), ((), ()))


def _dot(a, b):
    return jnp.dot(a, b, preferred_element_type=f32)


def _dot_nt(a, b):
    return lax.dot_general(a, b, NT, preferred_element_type=f32)


def _phi(t):
    return jnp.where(t > 0, t + 1.0, jnp.exp(t))


def _ln_tiles(xs):
    tot = xs[0]
    for x in xs[1:]:
        tot = tot + x
    mean = jnp.sum(tot, axis=-1, keepdims=True) * (1.0 / D)
    ds = [x - mean for x in xs]
    sq = ds[0] * ds[0]
    for d in ds[1:]:
        sq = sq + d * d
    var = jnp.sum(sq, axis=-1, keepdims=True) * (1.0 / D)
    rstd = lax.rsqrt(var + EPS)
    return [d * rstd for d in ds]


def _kernel(x_hbm, wq_hbm, wk_hbm, wv_hbm, wo_hbm, beta_ref, wr_ref, wg_hbm, wu_hbm, wd_hbm,
            out_hbm,
            XIO, X, XN, XB, WQ, WK, WV, WO, WG, WU, WD,
            QS, PQ, KK, PK, VT, OO, MT, MTB, ZZ, ZB, ZC, GATE, TOP,
            sem_x, sem_w, sem_f, sem_o, sem_p):
    def x_copy(s, n):
        return pltpu.make_async_copy(
            x_hbm.at[pl.ds(s * L, L), pl.ds(n * 128, 128)], XIO.at[n, pl.ds(s * L, L), :], sem_x.at[s])

    def w_copy(w_hbm, buf, i, n):
        return pltpu.make_async_copy(w_hbm.at[:, pl.ds(n * 128, 128)], buf.at[n], sem_w.at[i, n])

    def f_copy(w_hbm, buf, i, n):
        return pltpu.make_async_copy(w_hbm.at[:, pl.ds(n * 128, 128)], buf.at[n], sem_f.at[i])

    for n in range(NG):
        x_copy(0, n).start()
    for n in range(NG):
        w_copy(wq_hbm, WQ, 0, n).start()
        w_copy(wk_hbm, WK, 1, n).start()
        w_copy(wv_hbm, WV, 2, n).start()
    for s in range(1, NSEG):
        for n in range(NG):
            x_copy(s, n).start()
    for n in range(NG):
        w_copy(wo_hbm, WO, 3, n).start()
    for n in range(NF):
        f_copy(wg_hbm, WG, 0, n).start()
    for n in range(NF):
        f_copy(wu_hbm, WU, 1, n).start()
    for n in range(NG):
        f_copy(wd_hbm, WD, 2, n).start()

    lane = lax.broadcasted_iota(i32, (128, 128), 1)
    row = lax.broadcasted_iota(i32, (128, 128), 0)
    causal = row <= lane
    blockdiag = (row // DH) == (lane // DH)
    lane64 = lax.broadcasted_iota(i32, (64, 128), 1)
    hmask = [jnp.where((lane64 >= h * DH) & (lane64 < (h + 1) * DH), u32(0xFFFFFFFF), u32(0)) for h in range(4)]
    lane8 = lax.broadcasted_iota(i32, (8, 128), 1)
    sub8 = lax.broadcasted_iota(i32, (8, 128), 0)

    gv = jax.nn.sigmoid(beta_ref[...].astype(f32))
    for h in range(H):
        GATE[h] = gv[0, h]

    def first_ln(s):
        for n in range(NG):
            x_copy(s, n).wait()

        def body(c, carry):
            r0 = pl.multiple_of(s * L + c * CH, CH)
            xs = [XIO[n, pl.ds(r0, CH), :].astype(f32) for n in range(NG)]
            for n in range(NG):
                X[n, pl.ds(r0, CH), :] = xs[n]
            ys = _ln_tiles(xs)
            for n in range(NG):
                XN[n, pl.ds(r0, CH), :] = ys[n].astype(bf16)
            return carry
        lax.fori_loop(0, NG, body, 0)

    def xn_lhs(s):
        r0 = pl.multiple_of(s * L, L)
        return jnp.concatenate([XN[k, pl.ds(r0, L), :] for k in range(NG)], axis=1)

    def q_proj(s, g, par, need_phi):
        q = _dot(xn_lhs(s), WQ[g])
        QS[par, g] = (q * QSCALE).astype(bf16)
        if need_phi:
            PQ[par, g] = _phi(q).astype(bf16)

    def k_proj(s, g, par, need_phi):
        k = _dot(xn_lhs(s), WK[g])
        KK[par, g] = k.astype(bf16)
        if need_phi:
            pk = _phi(k)
            PK[par, g] = pk.astype(bf16)
            ZC[par, g] = jnp.sum(pk.reshape(L // 8, 8, 128), axis=0)

    def v_proj(s, g, par):
        v = _dot(xn_lhs(s), WV[g]).astype(bf16)
        for j in range(4):
            VT[par, g, j] = v[j * 128:(j + 1) * 128, :].T

    def o_proj_ln(s, c, par, last_layer_flag):
        r0 = pl.multiple_of(s * L + c * CH, CH)
        cr = pl.multiple_of(c * CH, CH)
        lhs = jnp.concatenate([OO[par, k, pl.ds(cr, CH), :] for k in range(NG)], axis=1)
        rhs = jnp.concatenate([WO[n] for n in range(NG)], axis=1)
        att = _dot(lhs, rhs)
        x1 = [X[n, pl.ds(r0, CH), :] + att[:, n * 128:(n + 1) * 128] for n in range(NG)]
        xb = _ln_tiles(x1)
        acc = xb[0] * wr_ref[:, 0:128].astype(f32)
        for n in range(1, NG):
            acc = acc + xb[n] * wr_ref[:, n * 128:(n + 1) * 128].astype(f32)
        r = jnp.sum(acc, axis=-1, keepdims=True)
        r = jnp.broadcast_to(r, (CH, 128))
        m1, i1, m2, i2 = TOP[0], TOP[1], TOP[2], TOP[3]
        for t in range(CH // 8):
            rv = r[t * 8:(t + 1) * 8, :]
            iv = (sub8 + (r0 + t * 8)).astype(f32)
            g1 = rv > m1
            g2 = rv > m2
            m2 = jnp.where(g1, m1, jnp.where(g2, rv, m2))
            i2 = jnp.where(g1, i1, jnp.where(g2, iv, i2))
            m1 = jnp.where(g1, rv, m1)
            i1 = jnp.where(g1, iv, i1)
        TOP[0] = m1
        TOP[1] = i1
        TOP[2] = m2
        TOP[3] = i2
        x2 = [x1[n] + xb[n] for n in range(NG)]
        for n in range(NG):
            X[n, pl.ds(r0, CH), :] = x2[n]
            XB[n, pl.ds(r0, CH), :] = xb[n].astype(bf16)
            XIO[n, pl.ds(r0, CH), :] = x2[n].astype(bf16)
        xn = _ln_tiles(x2)
        for n in range(NG):
            XN[n, pl.ds(r0, CH), :] = xn[n].astype(bf16)

    def attention(g, par, has_mem, upd_mem, mid, late):
        def qk(i):
            qu = pltpu.bitcast(QS[par, g, pl.ds(i * 128, 128), :], u32)
            qm = jnp.concatenate([pltpu.bitcast(qu & hmask[h], bf16) for h in range(4)], axis=0)
            return _dot_nt(KK[par, g, pl.ds(0, (i + 1) * 128), :], qm)

        def sm(i, sT):
            nk = (i + 1) * 128
            sd = jnp.where(jnp.concatenate([causal] * 4, axis=1), sT[nk - 128:], NEG)
            sx = jnp.concatenate([sT[:nk - 128], sd], axis=0) if i > 0 else sd
            m = jnp.max(sx, axis=0, keepdims=True)
            p = jnp.exp2(sx - m)
            l = jnp.sum(p, axis=0, keepdims=True)
            return p.astype(bf16), l

        order = [3, 2, 1, 0]
        sts = {i: qk(i) for i in order}
        mid()
        if has_mem:
            lhs = jnp.concatenate([MTB[g], ZB[g]], axis=0)
            memT = _dot_nt(lhs, PQ[par, g])
        pls = {i: sm(i, sts[i]) for i in order}
        gates = [GATE[g * 4 + h] for h in range(4)]
        for i in order:
            p, l = pls[i]
            nk = (i + 1) * 128
            linv = 1.0 / l
            outs = []
            for h in range(4):
                vt = jnp.concatenate([VT[par, g, j, pl.ds(h * DH, DH), :] for j in range(i + 1)], axis=1)
                oT = _dot(vt, p[:, h * 128:(h + 1) * 128])
                o = oT * (linv[:, h * 128:(h + 1) * 128] * (1.0 - gates[h]))
                if has_mem:
                    num = memT[h * DH:(h + 1) * DH, i * 128:(i + 1) * 128]
                    den = memT[128 + h * 8:128 + (h + 1) * 8, i * 128:(i + 1) * 128] + 1e-6
                    w = gates[h] / den
                    o = o + num * jnp.concatenate([w] * 4, axis=0)
                outs.append(o)
            oT_all = jnp.concatenate(outs, axis=0).astype(bf16)
            OO[par, g, pl.ds(i * 128, 128), :] = oT_all.T
        if upd_mem:
            vt_all = jnp.concatenate([VT[par, g, j] for j in range(4)], axis=1)
            dm = _dot(vt_all, PK[par, g])
            mt = MT[g] + jnp.where(blockdiag, dm, 0.0)
            MT[g] = mt
            MTB[g] = mt.astype(bf16)
            z = ZZ[g] + jnp.sum(ZC[par, g], axis=0, keepdims=True)
            ZZ[g] = z
            ZB[g] = jnp.concatenate(
                [jnp.where((lane8 >= h * DH) & (lane8 < (h + 1) * DH), z, 0.0) for h in range(4)], axis=0).astype(bf16)
        late()

    def layer(li, carry):
        first = li == 0

        MT[...] = jnp.zeros(MT.shape, f32)
        ZZ[...] = jnp.zeros(ZZ.shape, f32)
        TOP[0] = jnp.full((8, 128), -jnp.inf, f32)
        TOP[1] = jnp.zeros((8, 128), f32)
        TOP[2] = jnp.full((8, 128), -jnp.inf, f32)
        TOP[3] = jnp.zeros((8, 128), f32)

        @pl.when(first)
        def _():
            first_ln(0)

        def pro(g, c):
            @pl.when(first)
            def _():
                pltpu.make_async_copy(WQ.at[g], WQ.at[g], sem_w.at[0, g]).wait()
                pltpu.make_async_copy(WK.at[g], WK.at[g], sem_w.at[1, g]).wait()
                pltpu.make_async_copy(WV.at[g], WV.at[g], sem_w.at[2, g]).wait()
            q_proj(0, g, 0, False)
            k_proj(0, g, 0, True)
            v_proj(0, g, 0)
            return c
        lax.fori_loop(0, NG, pro, 0)

        @pl.when(first)
        def _():
            for s in range(1, NSEG):
                first_ln(s)
            for n in range(NG):
                w_copy(wo_hbm, WO, 3, n).wait()

        def b0(g, c):
            attention(g, 0, False, True,
                      lambda: k_proj(1, g, 1, True),
                      lambda: (q_proj(1, g, 1, True), v_proj(1, g, 1)))
            return c
        lax.fori_loop(0, NG, b0, 0)

        def b1(it, c):
            s = 1 + it // NG
            g = it % NG
            par = s % 2
            o_proj_ln(s - 1, g, 1 - par, None)
            attention(g, par, True, True,
                      lambda: k_proj(s + 1, g, 1 - par, True),
                      lambda: (q_proj(s + 1, g, 1 - par, True), v_proj(s + 1, g, 1 - par)))
            return c
        lax.fori_loop(0, 2 * NG, b1, 0)

        def b3(g, c):
            attention(g, 1, True, False,
                      lambda: o_proj_ln(2, g, 0, None),
                      lambda: None)
            return c
        lax.fori_loop(0, NG, b3, 0)

        def epi(g, c):
            o_proj_ln(3, g, 1, None)
            return c
        lax.fori_loop(0, NG, epi, 0)

        def out_copy(n):
            return pltpu.make_async_copy(XIO.at[n], out_hbm.at[:, pl.ds(n * 128, 128)], sem_o.at[0])

        @pl.when(li == 1)
        def _():
            for n in range(NG):
                out_copy(n).start()

        m1, i1, m2, i2 = TOP[0], TOP[1], TOP[2], TOP[3]
        big = f32(1e9)
        ra = jnp.max(m1, axis=0, keepdims=True)
        ia = jnp.min(jnp.where(m1 == ra, i1, big), axis=0, keepdims=True)
        isa = i1 == ia
        cv = jnp.where(isa, m2, m1)
        ci = jnp.where(isa, i2, i1)
        rb = jnp.max(cv, axis=0, keepdims=True)
        ib = jnp.min(jnp.where(cv == rb, ci, big), axis=0, keepdims=True)
        idx = [ia.astype(i32)[0, 0], ib.astype(i32)[0, 0]]
        idx = [jnp.clip(t, 0, S - 1) for t in idx]
        row16 = lax.broadcasted_iota(i32, (16, 128), 0)
        gsel = jnp.where(row16 == 0, jax.nn.sigmoid(ra), jnp.where(row16 == 1, jax.nn.sigmoid(rb), 0.0))

        base = [pl.multiple_of((t // 16) * 16, 16) for t in idx]
        off = [t % 16 for t in idx]
        xsel = []
        for n in range(NG):
            rows = []
            for t in range(2):
                blk = XB[n, pl.ds(base[t], 16), :].astype(f32)
                rows.append(jnp.sum(jnp.where(row16 == off[t], blk, 0.0), axis=0, keepdims=True))
            xsel.append(jnp.where(row16 == 0, rows[0], jnp.where(row16 == 1, rows[1], 0.0)))
        xsel = jnp.concatenate(xsel, axis=1).astype(bf16)

        @pl.when(first)
        def _():
            pltpu.make_async_copy(WG, WG, sem_f.at[0]).wait()
            pltpu.make_async_copy(WU, WU, sem_f.at[1]).wait()
            pltpu.make_async_copy(WD, WD, sem_f.at[2]).wait()

        wg = jnp.concatenate([WG[n] for n in range(NF)], axis=1)
        wu = jnp.concatenate([WU[n] for n in range(NF)], axis=1)
        gg = _dot(xsel, wg)
        uu = _dot(xsel, wu)
        hh = (gg * jax.nn.sigmoid(gg) * uu).astype(bf16)
        wd = jnp.concatenate([WD[n] for n in range(NG)], axis=1)
        y = _dot(hh, wd)

        @pl.when(li == 1)
        def _():
            for n in range(NG):
                out_copy(n).wait()

        for t in range(2):
            b8 = pl.multiple_of((idx[t] // 8) * 8, 8)
            o8 = idx[t] % 8
            xs = []
            for n in range(NG):
                yt = y[:, n * 128:(n + 1) * 128] * gsel
                yrow = jnp.sum(jnp.where(row16 == t, yt, 0.0), axis=0, keepdims=True)
                blk = X[n, pl.ds(b8, 8), :]
                blk = jnp.where(sub8 == o8, blk + yrow, blk)
                X[n, pl.ds(b8, 8), :] = blk
                xs.append(blk)
            xn = _ln_tiles(xs)
            for n in range(NG):
                sel = row16 == off[t]
                new_x = jnp.sum(jnp.where(sub8 == o8, xs[n], 0.0), axis=0, keepdims=True)
                new_n = jnp.sum(jnp.where(sub8 == o8, xn[n], 0.0), axis=0, keepdims=True)
                blk = XN[n, pl.ds(base[t], 16), :]
                XN[n, pl.ds(base[t], 16), :] = jnp.where(sel, new_n, blk.astype(f32)).astype(bf16)
                blk = XIO[n, pl.ds(base[t], 16), :]
                XIO[n, pl.ds(base[t], 16), :] = jnp.where(sel, new_x, blk.astype(f32)).astype(bf16)

        @pl.when(li == 1)
        def _():
            for t in range(2):
                for n in range(NG):
                    cp = pltpu.make_async_copy(
                        XIO.at[n, pl.ds(base[t], 16), :],
                        out_hbm.at[pl.ds(base[t], 16), pl.ds(n * 128, 128)], sem_p.at[0])
                    cp.start()
                    cp.wait()
        return carry

    lax.fori_loop(0, 2, layer, 0)


def _build(interpret=False):
    any_spec = pl.BlockSpec(memory_space=pl.ANY)
    vmem_spec = pl.BlockSpec(memory_space=pltpu.VMEM)
    V = pltpu.VMEM
    scratch = [
        V((NG, S, 128), bf16),
        V((NG, S, 128), f32),
        V((NG, S, 128), bf16),
        V((NG, S, 128), bf16),
        V((NG, D, 128), bf16), V((NG, D, 128), bf16), V((NG, D, 128), bf16), V((NG, D, 128), bf16),
        V((NF, D, 128), bf16), V((NF, D, 128), bf16), V((NG, F, 128), bf16),
        V((2, NG, L, 128), bf16),
        V((2, NG, L, 128), bf16),
        V((2, NG, L, 128), bf16),
        V((2, NG, L, 128), bf16),
        V((2, NG, 4, 128, 128), bf16),
        V((2, NG, L, 128), bf16),
        V((NG, 128, 128), f32), V((NG, 128, 128), bf16),
        V((NG, 8, 128), f32), V((NG, 32, 128), bf16),
        V((2, NG, 8, 128), f32),
        pltpu.SMEM((H,), f32),
        V((4, 8, 128), f32),
        pltpu.SemaphoreType.DMA((NSEG,)),
        pltpu.SemaphoreType.DMA((4, NG)),
        pltpu.SemaphoreType.DMA((3,)),
        pltpu.SemaphoreType.DMA((1,)),
        pltpu.SemaphoreType.DMA((1,)),
    ]
    return pl.pallas_call(
        _kernel,
        out_shape=jax.ShapeDtypeStruct((S, D), bf16),
        in_specs=[any_spec] * 5 + [vmem_spec, vmem_spec] + [any_spec] * 3,
        out_specs=any_spec,
        scratch_shapes=scratch,
        compiler_params=pltpu.CompilerParams(vmem_limit_bytes=110 * 1024 * 1024),
        interpret=pltpu.InterpretParams() if interpret else False,
        name="infini_mod",
    )


@jax.jit
def pallas_interleave_layers__memory_aug_infini_attn__moe_arch_mod__prompt_kernel(
    A_x, A_wq, A_wk, A_wv, A_wo, A_beta, B_x, B_w_r, B_w_gate, B_w_up, B_w_down,
):
    del B_x
    out = _build()(A_x.reshape(S, D), A_wq, A_wk, A_wv, A_wo, A_beta.reshape(1, H), B_w_r.reshape(1, D),
                   B_w_gate, B_w_up, B_w_down)
    return out.reshape(1, S, D)
```

```python
import os

import jax
import jax.numpy as jnp
from jax import lax
import jax.experimental.pallas as pl
import jax.experimental.pallas.tpu as pltpu

S = 2048
D = 1024
NSEG = 4
L = S // NSEG
H = 32
DH = D // H
NG = 8
F = 3584
NF = F // 128
CH = L // NG
EPS = 1e-5
LOG2E = 1.4426950408889634
QSCALE = (DH ** -0.5) * LOG2E
NEG = -1e30

SM = lambda i: " ".join(f"sm.{i}.{h}" for h in range(4))
LN = "ln.0@1 ln.1@0 ln.2@0 ln.3@0"
ORD_FULL = os.environ.get("ORD_FULL", f"qk.3 mem o.0.8 {LN} {SM(3)} pv.3 qk.2 k.0.4 {SM(2)} pv.2 qk.1 qk.0 q.0.4 {SM(1)} {SM(0)} pv.1 pv.0 v.0.4 upd")
ORD_FIRST = os.environ.get("ORD_FIRST", f"qk.3 k.0.4 {SM(3)} pv.3 qk.2 q.0.4 {SM(2)} pv.2 qk.1 qk.0 v.0.4 {SM(1)} {SM(0)} pv.1 pv.0 upd")
ORD_LAST = os.environ.get("ORD_LAST", f"qk.3 mem o.0 {SM(3)} qk.2 o.2 pv.3 {SM(2)} qk.1 o.4 pv.2 qk.0 o.6 {LN} {SM(1)} {SM(0)} pv.1 pv.0")
ORD_PRO = os.environ.get("ORD_PRO", "v.0.4 k.0.4 q.0.4")
ORD_EPI = os.environ.get("ORD_EPI", "lp.0.4@0 o.0.8@0")
ORD_EPI2 = os.environ.get("ORD_EPI2", "lp.0.4@0")
ORD_PRO0 = os.environ.get("ORD_PRO0", "v.0.4 f.T.0 k.0.4 f.T.1 f.T.2 q.0.4 f.T.3")
LAG = int(os.environ.get("LAG", "2"))
MINI = os.environ.get("MINI", "")
NOMAX = int(os.environ.get("NOMAX", "0"))
UNROLL = int(os.environ.get("UNROLL", "1"))

bf16 = jnp.bfloat16
f32 = jnp.float32
u32 = jnp.uint32
i32 = jnp.int32
NT = (((1,), (1,)), ((), ()))


def _al(i, m):
    return i if isinstance(i, int) else pl.multiple_of(i, m)


def _dot(a, b):
    return jnp.dot(a, b, preferred_element_type=f32)


def _dot_nt(a, b):
    return lax.dot_general(a, b, NT, preferred_element_type=f32)


def _phi(t):
    return jnp.where(t > 0, t + 1.0, jnp.exp(t))


def _ln_tiles(xs):
    tot = xs[0]
    for x in xs[1:]:
        tot = tot + x
    mean = jnp.sum(tot, axis=-1, keepdims=True) * (1.0 / D)
    ds = [x - mean for x in xs]
    sq = ds[0] * ds[0]
    for d in ds[1:]:
        sq = sq + d * d
    var = jnp.sum(sq, axis=-1, keepdims=True) * (1.0 / D)
    rstd = lax.rsqrt(var + EPS)
    return [d * rstd for d in ds]


def _kernel(x_hbm, wq_hbm, wk_hbm, wv_hbm, wo_hbm, beta_ref, wr_ref, wg_hbm, wu_hbm, wd_hbm,
            out_hbm, *scr):
    scr = list(scr)

    def take(n):
        out = scr[:n]
        del scr[:n]
        return out
    XIO, X, XN, XB = take(NSEG), take(NSEG), take(NSEG), take(NSEG)
    QS, PQ, KK, PK, VT, OO, ZC = take(2), take(2), take(2), take(2), take(2), take(2), take(2)
    SS, PP = take(4), take(4)
    (WQ, WK, WV, WO, WG, WU, WD, MT, MTB, ZZ, ZB, GATE, ZO, TOP, SEL, WR,
     sem_x, sem_w, sem_f, sem_o, sem_p) = scr

    def x_copy(s, n):
        return pltpu.make_async_copy(
            x_hbm.at[pl.ds(s * L, L), pl.ds(n * 128, 128)], XIO[s].at[n], sem_x.at[s])

    def w_copy(w_hbm, buf, i, n):
        return pltpu.make_async_copy(w_hbm.at[:, pl.ds(_al(n * 128, 128), 128)], buf.at[n], sem_w.at[i, n])

    def f_copy(w_hbm, buf, i, n):
        return pltpu.make_async_copy(w_hbm.at[:, pl.ds(_al(n * 128, 128), 128)], buf.at[n], sem_f.at[i])

    _sc0 = jax.named_scope("s_dmastart"); _sc0.__enter__()
    def start_w(n):
        w_copy(wv_hbm, WV, 2, n).start()
        w_copy(wk_hbm, WK, 1, n).start()
        w_copy(wq_hbm, WQ, 0, n).start()

    for s in range(NSEG):
        for n in range(NG):
            x_copy(s, n).start()
        start_w(2 * s)
        start_w(2 * s + 1)

    _sc0.__exit__(None, None, None)
    def late_copies(g):
        cps = [f_copy(wd_hbm, WD, 2, g)]
        for w_hbm, buf, i in ((wg_hbm, WG, 0), (wu_hbm, WU, 1)):
            for t in range(3):
                cps.append(f_copy(w_hbm, buf, i, g + NG * t))
            r0 = _al((g % 2) * (D // 2), D // 2)
            n = 3 * NG + g // 2
            cps.append(pltpu.make_async_copy(
                w_hbm.at[pl.ds(r0, D // 2), pl.ds(_al(n * 128, 128), 128)],
                buf.at[n, pl.ds(r0, D // 2), :], sem_f.at[i]))
        return cps

    lane = lax.broadcasted_iota(i32, (128, 128), 1)
    row = lax.broadcasted_iota(i32, (128, 128), 0)
    causal = row <= lane
    blockdiag = (row // DH) == (lane // DH)
    lane64 = lax.broadcasted_iota(i32, (64, 128), 1)
    hmask = [jnp.where((lane64 >= h * DH) & (lane64 < (h + 1) * DH), u32(0xFFFFFFFF), u32(0)) for h in range(4)]
    lane8 = lax.broadcasted_iota(i32, (8, 128), 1)
    sub8 = lax.broadcasted_iota(i32, (8, 128), 0)

    _sc1 = jax.named_scope("s_consts"); _sc1.__enter__()
    ZO[0] = 0
    ZO[1] = 0
    gv = jax.nn.sigmoid(beta_ref[...].astype(f32))
    for h in range(H):
        GATE[h] = gv[0, h]

    for n in range(NG):
        WR[n] = jnp.broadcast_to(wr_ref[:, n * 128:(n + 1) * 128].astype(f32), (8, 128))

    _sc1.__exit__(None, None, None)
    def first_ln(t, r0, rows):
        xs = [XIO[t][n, pl.ds(r0, rows), :].astype(f32) for n in range(NG)]
        for n in range(NG):
            X[t][n, pl.ds(r0, rows), :] = xs[n]
        ys = _ln_tiles(xs)
        for n in range(NG):
            XN[t][n, pl.ds(r0, rows), :] = ys[n].astype(bf16)

    def body(s, g, order, has_mem=False, u=0):
        par = s % 2
        z0, z1 = ZO[0], ZO[1]
        marks = []
        st = {"m": {}, "l": {}, "mem": None, "zc": None}
        gates = [GATE[g * 4 + h] for h in range(4)]

        def anchor(lag, *refs):
            lag = min(lag, len(marks))
            if lag == 0:
                return
            mk = marks[-lag]
            for ref in refs:
                slot = ref.shape[0] - 1
                if ref.dtype == f32:
                    val = mk
                else:
                    val = jnp.concatenate([mk, mk], axis=0).astype(ref.dtype)
                idx = (slot + z0,) + (0,) * (len(ref.shape) - 3) + (pl.ds(0, val.shape[0]), slice(None))
                ref[idx] = val

        def xn_lhs(t, c, nc):
            return jnp.concatenate([XN[t][k, pl.ds(c * 128, nc * 128), :] for k in range(NG)], axis=1)

        def q_proj(lag, c, nc=1):
            t, tp = s + 1, 1 - par
            anchor(lag, XN[t], WQ)
            q = _dot(xn_lhs(t, c, nc), WQ[g])
            marks.append(q[0:8])
            rows = pl.ds(c * 128, nc * 128)
            QS[tp][g, rows, :] = (q * QSCALE).astype(bf16)
            PQ[tp][g, rows, :] = _phi(q).astype(bf16)

        def k_proj(lag, c, nc=1):
            t, tp = s + 1, 1 - par
            anchor(lag, XN[t], WK)
            k = _dot(xn_lhs(t, c, nc), WK[g])
            marks.append(k[0:8])
            rows = pl.ds(c * 128, nc * 128)
            KK[tp][g, rows, :] = k.astype(bf16)
            pk = _phi(k)
            PK[tp][g, rows, :] = pk.astype(bf16)
            zc = st["zc"]
            for r in range(nc * 16):
                zc = pk[r * 8:(r + 1) * 8] if zc is None else zc + pk[r * 8:(r + 1) * 8]
            st["zc"] = zc
            if c + nc == 4:
                ZC[tp][g] = zc

        def v_proj(lag, c, nc=1):
            t, tp = s + 1, 1 - par
            anchor(lag, XN[t], WV)
            v = _dot(xn_lhs(t, c, nc), WV[g])
            marks.append(v[0:8])
            v = v.astype(bf16)
            for j in range(nc):
                VT[tp][g, c + j] = v[j * 128:(j + 1) * 128, :].T

        def o_proj(lag, n0, nn=2):
            t, tp = s - 1, 1 - par
            cr = _al(g * CH, CH)
            anchor(lag, OO[tp], WO)
            lhs = jnp.concatenate([OO[tp][k, pl.ds(cr, CH), :] for k in range(NG)], axis=1)
            rhs = jnp.concatenate([WO[n] for n in range(n0, n0 + nn)], axis=1)
            att = _dot(lhs, rhs)
            marks.append(att[0:8, 0:128])
            for i in range(nn):
                n = n0 + i
                X[t][n + z0, pl.ds(cr, CH), :] = X[t][n, pl.ds(cr, CH), :] + att[:, i * 128:(i + 1) * 128]

        def o_lp(lag, c, nc=1):
            if g > 0:
                o_ln(lag, c, nc, g - 1)

        def o_ln(lag, c, nc=1, g=g):
            t = s - 1
            anchor(lag, X[t])
            R = 16 * nc
            r0 = _al(g * CH + c * 16, 16)
            x1 = [X[t][n + z1, pl.ds(r0, R), :] for n in range(NG)]
            xb = _ln_tiles(x1)
            wr = [jnp.concatenate([WR[n]] * (R // 8), axis=0) for n in range(NG)]
            acc = xb[0] * wr[0]
            for n in range(1, NG):
                acc = acc + xb[n] * wr[n]
            r = jnp.broadcast_to(jnp.sum(acc, axis=-1, keepdims=True), (R, 128))
            m1, i1, m2, i2 = TOP[0], TOP[1], TOP[2], TOP[3]
            for u in range(R // 8):
                rv = r[u * 8:(u + 1) * 8, :]
                iv = (sub8 + (r0 + (t * L + u * 8))).astype(f32)
                g1 = rv > m1
                g2 = rv > m2
                m2 = jnp.where(g1, m1, jnp.where(g2, rv, m2))
                i2 = jnp.where(g1, i1, jnp.where(g2, iv, i2))
                m1 = jnp.where(g1, rv, m1)
                i1 = jnp.where(g1, iv, i1)
            TOP[0] = m1
            TOP[1] = i1
            TOP[2] = m2
            TOP[3] = i2
            x2 = [x1[n] + xb[n] for n in range(NG)]
            for n in range(NG):
                X[t][n, pl.ds(r0, R), :] = x2[n]
                XB[t][n, pl.ds(r0, R), :] = xb[n].astype(bf16)
                XIO[t][n, pl.ds(r0, R), :] = x2[n].astype(bf16)
            xn = _ln_tiles(x2)
            for n in range(NG):
                XN[t][n, pl.ds(r0, R), :] = xn[n].astype(bf16)

        def qk(lag, i):
            nk = (i + 1) * 128
            anchor(lag, QS[par], KK[par])
            qu = pltpu.bitcast(QS[par][g, pl.ds(i * 128, 128), :], u32)
            qm = jnp.concatenate([pltpu.bitcast(qu & hmask[h], bf16) for h in range(4)], axis=0)
            sT = _dot_nt(KK[par][g, pl.ds(0, nk), :], qm)
            marks.append(sT[0:8, 0:128])
            if NOMAX:
                for h in range(4):
                    l = None
                    for r in range(nk // 16):
                        t = sT[r * 16:(r + 1) * 16, h * 128:(h + 1) * 128]
                        if r >= i * 8:
                            t = jnp.where(causal[(r - i * 8) * 16:(r - i * 8 + 1) * 16], t, NEG)
                        e = jnp.exp2(t)
                        es = e[0:8] + e[8:16]
                        l = es if l is None else l + es
                        PP[i][h + z0, pl.ds(r * 16, 16), :] = e.astype(bf16)
                    st["l"][(i, h)] = jnp.sum(l, axis=0, keepdims=True)
                return
            for h in range(4):
                mx = None
                for r in range(nk // 8):
                    t = sT[r * 8:(r + 1) * 8, h * 128:(h + 1) * 128]
                    if r >= i * 16:
                        t = jnp.where(causal[(r - i * 16) * 8:(r - i * 16 + 1) * 8], t, NEG)
                    mx = t if mx is None else jnp.maximum(mx, t)
                    SS[i][h + z0, pl.ds(r * 8, 8), :] = t
                st["m"][(i, h)] = jnp.max(mx, axis=0, keepdims=True)

        def sm(lag, i, h0, nh=1):
            if NOMAX:
                return
            nk = (i + 1) * 128
            anchor(lag, SS[i])
            for h in range(h0, h0 + nh):
                m = st["m"][(i, h)]
                la = [None, None]
                for r in range(nk // 16):
                    e = jnp.exp2(SS[i][h + z1, pl.ds(r * 16, 16), :] - m)
                    es = e[0:8] + e[8:16]
                    la[r % 2] = es if la[r % 2] is None else la[r % 2] + es
                    PP[i][h + z0, pl.ds(r * 16, 16), :] = e.astype(bf16)
                st["l"][(i, h)] = jnp.sum(la[0] + la[1], axis=0, keepdims=True)

        def mem(lag):
            anchor(lag, MTB, PQ[par])
            lhs = jnp.concatenate([MTB[g], ZB[g]], axis=0)
            st["mem"] = _dot_nt(lhs, PQ[par][g])
            marks.append(st["mem"][0:8, 0:128])

        def pv(lag, i):
            nk = (i + 1) * 128
            anchor(lag, VT[par], PP[i])
            outs = []
            for h in range(4):
                vt = jnp.concatenate([VT[par][g, j, pl.ds(h * DH, DH), :] for j in range(i + 1)], axis=1)
                oT = _dot(vt, PP[i][h + z1])
                if h == 0:
                    marks.append(oT[0:8])
                o = oT * ((1.0 - gates[h]) / st["l"][(i, h)])
                if has_mem:
                    memT = st["mem"]
                    num = memT[h * DH:(h + 1) * DH, i * 128:(i + 1) * 128]
                    den = memT[128 + h * 8:128 + (h + 1) * 8, i * 128:(i + 1) * 128] + 1e-6
                    w = gates[h] / den
                    o = o + num * jnp.concatenate([w] * 4, axis=0)
                outs.append(o)
            oT_all = jnp.concatenate(outs, axis=0).astype(bf16)
            OO[par][g, pl.ds(i * 128, 128), :] = oT_all.T

        def upd(lag):
            anchor(lag, VT[par], PK[par])
            vt_all = jnp.concatenate([VT[par][g, j] for j in range(4)], axis=1)
            dm = _dot(vt_all, PK[par][g])
            marks.append(dm[0:8])
            mt = MT[g] + jnp.where(blockdiag, dm, 0.0)
            MT[g] = mt
            MTB[g] = mt.astype(bf16)
            z = ZZ[g] + jnp.sum(ZC[par][g], axis=0, keepdims=True)
            ZZ[g] = z
            ZB[g] = jnp.concatenate(
                [jnp.where((lane8 >= h * DH) & (lane8 < (h + 1) * DH), z, 0.0) for h in range(4)], axis=0).astype(bf16)

        def fln(lag, t, c):
            first_ln(t, _al((g - 2 * t) * 256 + c * 64, 64), 64)

        table = {"lp": o_lp, "f": fln, "qk": qk, "sm": sm, "pv": pv, "mem": mem, "upd": upd,
                 "o": o_proj, "ln": o_ln, "q": q_proj, "k": k_proj, "v": v_proj}
        for kind, args, lag in order:
            table[kind](lag, *args)

    def parse(txt, drop=()):
        out = []
        for w in txt.split():
            lag = LAG
            if "@" in w:
                w, lg = w.split("@")
                lag = int(lg)
            p = w.split(".")
            if p[0] not in drop:
                out.append((p[0], tuple(int(x) for x in p[1:]), lag))
        return out

    FULL = parse(ORD_FULL)
    FIRST = parse(ORD_FIRST)
    LAST = parse(ORD_LAST)
    PRO = parse(ORD_PRO)
    EPI = parse(ORD_EPI)
    EPI2 = parse(ORD_EPI2)

    if MINI:
        order, hm, sg = {"full": (FULL, True, 1), "first": (FIRST, False, 0), "last": (LAST, True, 3),
                         "pro": (PRO, False, -1), "epi": (EPI, False, 4)}[MINI]

        def b(g, c):
            for u in range(UNROLL):
                body(sg, g * UNROLL + u, order, hm)
            return c
        lax.fori_loop(0, NG // UNROLL, b, 0)
        return

    with jax.named_scope("s_xwait0"):
        for n in range(NG):
            x_copy(0, n).wait()

    def ln0(c, carry):
        first_ln(0, _al(c * CH, CH), CH)
        return carry
    with jax.named_scope("s_ln0"):
        lax.fori_loop(0, NG, ln0, 0)

    for t in range(NSEG):
        if t > 0:
          with jax.named_scope(f"s_xwait{t}"):
            for n in range(NG):
                x_copy(t, n).wait()

        if t == 2:
            for n in range(NG):
                w_copy(wo_hbm, WO, 3, n).start()

        def pro0(g, c, t=t):
            for i, w in ((2, WV), (1, WK), (0, WQ)):
                pltpu.make_async_copy(w.at[g], w.at[g], sem_w.at[i, g]).wait()
            body(-1, g, PRO if t == 0 else parse(ORD_PRO0.replace("T", str(t))))
            return c
        with jax.named_scope(f"s_pro0_{t}"):
            lax.fori_loop(2 * t, 2 * t + 2, pro0, 0)

    for n in range(NG):
        w_copy(wo_hbm, WO, 3, n).wait()

    def layer(li, carry):
        _sc2 = jax.named_scope("s_reset"); _sc2.__enter__()
        MT[...] = jnp.zeros(MT.shape, f32)
        ZZ[...] = jnp.zeros(ZZ.shape, f32)
        TOP[0] = jnp.full((8, 128), -jnp.inf, f32)
        TOP[1] = jnp.zeros((8, 128), f32)
        TOP[2] = jnp.full((8, 128), -jnp.inf, f32)
        TOP[3] = jnp.zeros((8, 128), f32)

        _sc2.__exit__(None, None, None)
        def out_copy(s, n):
            return pltpu.make_async_copy(
                XIO[s].at[n], out_hbm.at[pl.ds(s * L, L), pl.ds(n * 128, 128)], sem_o.at[0])

        def loop(s, order, has_mem, extra=None):
            def b(g, c):
                for u in range(UNROLL):
                    if extra is not None:
                        extra(g * UNROLL + u)
                    body(s, g * UNROLL + u, order, has_mem, u)
                return c
            with jax.named_scope(f"s_loop{s}"):
                lax.fori_loop(0, NG // UNROLL, b, 0)

        def start_late(g):
            for cp in late_copies(g):
                cp.start()

        def flush(s):
            @pl.when(li == 1)
            def _():
                for n in range(NG):
                    out_copy(s, n).start()

        loop(0, FIRST, False, start_late)
        loop(1, FULL, True)
        loop(2, FULL, True)
        flush(0)
        loop(3, LAST, True)
        flush(1)
        flush(2)
        with jax.named_scope("s_epi"):
            for c in range(NG + 1):
                body(4, c, EPI if c < NG else EPI2)
        flush(3)

        _sc = jax.named_scope('s_top2'); _sc.__enter__()
        m1, i1, m2, i2 = TOP[0], TOP[1], TOP[2], TOP[3]
        big = f32(1e9)
        ra = jnp.max(m1, axis=0, keepdims=True)
        ia = jnp.min(jnp.where(m1 == ra, i1, big), axis=0, keepdims=True)
        isa = i1 == ia
        cv = jnp.where(isa, m2, m1)
        ci = jnp.where(isa, i2, i1)
        rb = jnp.max(cv, axis=0, keepdims=True)
        ib = jnp.min(jnp.where(cv == rb, ci, big), axis=0, keepdims=True)
        idx = [ia.astype(i32)[0, 0], ib.astype(i32)[0, 0]]
        idx = [jnp.clip(t, 0, S - 1) for t in idx]
        row16 = lax.broadcasted_iota(i32, (16, 128), 0)
        gsel = jnp.where(row16 == 0, jax.nn.sigmoid(ra), jnp.where(row16 == 1, jax.nn.sigmoid(rb), 0.0))

        seg = [t // L for t in idx]
        loc = [t % L for t in idx]
        base = [pl.multiple_of((t // 16) * 16, 16) for t in loc]
        off = [t % 16 for t in loc]
        for t in range(2):
            for s in range(NSEG):
                @pl.when(seg[t] == s)
                def _(t=t, s=s):
                    for n in range(NG):
                        blk = XB[s][n, pl.ds(base[t], 16), :].astype(f32)
                        SEL[t, n] = jnp.broadcast_to(
                            jnp.sum(jnp.where(row16 == off[t], blk, 0.0), axis=0, keepdims=True), (8, 128))
        xsel = []
        for n in range(NG):
            r0_ = SEL[0, n][0:1]
            r1_ = SEL[1, n][0:1]
            xsel.append(jnp.where(row16 == 0, r0_, jnp.where(row16 == 1, r1_, 0.0)))
        xsel = jnp.concatenate(xsel, axis=1).astype(bf16)

        _sc.__exit__(None, None, None)
        _sc = jax.named_scope('s_ffn'); _sc.__enter__()
        pltpu.make_async_copy(WG, WG, sem_f.at[0]).wait()
        pltpu.make_async_copy(WU, WU, sem_f.at[1]).wait()
        pltpu.make_async_copy(WD, WD, sem_f.at[2]).wait()

        wg = jnp.concatenate([WG[n] for n in range(NF)], axis=1)
        wu = jnp.concatenate([WU[n] for n in range(NF)], axis=1)
        gg = _dot(xsel, wg)
        uu = _dot(xsel, wu)
        hh = (gg * jax.nn.sigmoid(gg) * uu).astype(bf16)
        wd = jnp.concatenate([WD[n] for n in range(NG)], axis=1)
        y = _dot(hh, wd)

        _sc.__exit__(None, None, None)
        _sc = jax.named_scope('s_fix'); _sc.__enter__()
        @pl.when(li == 1)
        def _():
            for s in range(NSEG):
                for n in range(NG):
                    out_copy(s, n).wait()

        for t in range(2):
            b8 = pl.multiple_of((loc[t] // 8) * 8, 8)
            o8 = loc[t] % 8
            yrows = []
            for n in range(NG):
                yt = y[:, n * 128:(n + 1) * 128] * gsel
                yrows.append(jnp.sum(jnp.where(row16 == t, yt, 0.0), axis=0, keepdims=True))
            for s in range(NSEG):
                @pl.when(seg[t] == s)
                def _(t=t, s=s, b8=b8, o8=o8, yrows=yrows):
                    xs = []
                    for n in range(NG):
                        blk = X[s][n, pl.ds(b8, 8), :]
                        blk = jnp.where(sub8 == o8, blk + yrows[n], blk)
                        X[s][n, pl.ds(b8, 8), :] = blk
                        xs.append(blk)
                    xn = _ln_tiles(xs)
                    sel = row16 == off[t]
                    for n in range(NG):
                        new_x = jnp.sum(jnp.where(sub8 == o8, xs[n], 0.0), axis=0, keepdims=True)
                        new_n = jnp.sum(jnp.where(sub8 == o8, xn[n], 0.0), axis=0, keepdims=True)
                        blk = XN[s][n, pl.ds(base[t], 16), :]
                        XN[s][n, pl.ds(base[t], 16), :] = jnp.where(sel, new_n, blk.astype(f32)).astype(bf16)
                        blk = XIO[s][n, pl.ds(base[t], 16), :]
                        XIO[s][n, pl.ds(base[t], 16), :] = jnp.where(sel, new_x, blk.astype(f32)).astype(bf16)

                    @pl.when(li == 1)
                    def _():
                        cps = [pltpu.make_async_copy(
                            XIO[s].at[n, pl.ds(base[t], 16), :],
                            out_hbm.at[pl.ds(s * L + base[t], 16), pl.ds(n * 128, 128)], sem_p.at[0])
                            for n in range(NG)]
                        for cp in cps:
                            cp.start()
                        for cp in cps:
                            cp.wait()
        _sc.__exit__(None, None, None)

        @pl.when(li == 0)
        def _():
            def pro(g, c):
                body(-1, g, PRO)
                return c
            with jax.named_scope("s_pro"):
                lax.fori_loop(0, NG, pro, 0)
        return carry

    lax.fori_loop(0, 2, layer, 0)


def _build(interpret=False):
    any_spec = pl.BlockSpec(memory_space=pl.ANY)
    vmem_spec = pl.BlockSpec(memory_space=pltpu.VMEM)
    V = pltpu.VMEM
    A = NG + 1
    scratch = (
        [V((NG, L, 128), bf16)] * NSEG + [V((A, L, 128), f32)] * NSEG
        + [V((A, L, 128), bf16)] * NSEG + [V((NG, L, 128), bf16)] * NSEG
        + [V((A, L, 128), bf16)] * 8
        + [V((A, 4, 128, 128), bf16)] * 2
        + [V((A, L, 128), bf16)] * 2
        + [V((NG, 8, 128), f32)] * 2
        + [V((5, (i + 1) * 128, 128), f32) for i in range(4)]
        + [V((5, (i + 1) * 128, 128), bf16) for i in range(4)]
    ) + [
        V((A, D, 128), bf16), V((A, D, 128), bf16), V((A, D, 128), bf16), V((A, D, 128), bf16),
        V((NF, D, 128), bf16), V((NF, D, 128), bf16), V((NG, F, 128), bf16),
        V((NG, 128, 128), f32), V((A, 128, 128), bf16),
        V((NG, 8, 128), f32), V((NG, 32, 128), bf16),
        pltpu.SMEM((H,), f32),
        pltpu.SMEM((2,), i32),
        V((4, 8, 128), f32),
        V((2, NG, 8, 128), f32),
        V((NG, 8, 128), f32),
        pltpu.SemaphoreType.DMA((NSEG,)),
        pltpu.SemaphoreType.DMA((4, NG)),
        pltpu.SemaphoreType.DMA((3,)),
        pltpu.SemaphoreType.DMA((1,)),
        pltpu.SemaphoreType.DMA((1,)),
    ]
    return pl.pallas_call(
        _kernel,
        out_shape=jax.ShapeDtypeStruct((S, D), bf16),
        in_specs=[any_spec] * 5 + [vmem_spec, vmem_spec] + [any_spec] * 3,
        out_specs=any_spec,
        scratch_shapes=scratch,
        compiler_params=pltpu.CompilerParams(vmem_limit_bytes=110 * 1024 * 1024, flags=(__import__("json").loads(os.environ.get("KFLAGS", "{}")) or None)),
        interpret=pltpu.InterpretParams() if interpret else False,
        name="infini_mod",
    )


@jax.jit
def pallas_interleave_layers__memory_aug_infini_attn__moe_arch_mod__prompt_kernel(
    A_x, A_wq, A_wk, A_wv, A_wo, A_beta, B_x, B_w_r, B_w_gate, B_w_up, B_w_down,
):
    del B_x
    out = _build()(A_x.reshape(S, D), A_wq, A_wk, A_wv, A_wo, A_beta.reshape(1, H), B_w_r.reshape(1, D),
                   B_w_gate, B_w_up, B_w_down)
    return out.reshape(1, S, D)
```

```python
import os

import jax
import jax.numpy as jnp
from jax import lax
import jax.experimental.pallas as pl
import jax.experimental.pallas.tpu as pltpu

S = 2048
D = 1024
NSEG = 4
L = S // NSEG
H = 32
DH = D // H
NG = 8
F = 3584
NF = F // 128
CH = L // NG
EPS = 1e-5
LOG2E = 1.4426950408889634
QSCALE = (DH ** -0.5) * LOG2E
NEG = -1e30

SM = lambda i: " ".join(f"sm.{i}.{h}" for h in range(4))
LN = "ln.0@1 ln.1@0 ln.2@0 ln.3@0"
ORD_FULL = os.environ.get("ORD_FULL", "o.0.8@0 qk.3@3 qk.0@0 ln.0.1@3 k.0.4 ln.1.1@1 qk.2@0 sm.3.2.2@0 ln.2.2@0 mem@2 qk.1@2 sm.3.0.2@2 v.0.4 pv.3@0 sm.2.2.2@2 sm.2.0.1@2 sm.2.1.1@2 sm.1.0.4@0 pv.2 sm.0.0.4@1 pv.1@2 pv.0@3 q.0.4@0 upd")
ORD_FIRST = os.environ.get("ORD_FIRST", "qk.2@2 k.0.4@0 qk.1@3 sm.2.1.3@0 sm.1.0.1@0 v.0.1@0 sm.2.0.1@3 sm.1.1.1@0 qk.3@2 sm.1.2.2@0 q.0.2@0 sm.3.0.4@1 upd@0 qk.0@2 v.3.1@0 sm.0.2.2@3 v.2.1@0 sm.0.0.2@0 v.1.1@3 pv.3@0 pv.0@3 pv.2@3 pv.1@0 q.2.2@0")
ORD_LAST = os.environ.get("ORD_LAST", "qk.2@2 qk.3@2 sm.2.0.1@2 sm.2.2.2@2 sm.2.1.1@2 qk.1@1 sm.3.0.4@2 lp.0.4@3 sm.1.1.1@0 mem@0 sm.1.0.1@3 o.0.4@0 sm.1.3.1@0 qk.0@2 sm.1.2.1@0 pv.2 sm.0.0.4@0 pv.3@3 pv.1@0 pv.0@2 o.4.4@0")
ORD_PRO = os.environ.get("ORD_PRO", "v.0.4 q.0.4@0 k.0.1@0 k.1.1@0 k.2.2@0")
ORD_EPI = os.environ.get("ORD_EPI", "lp.0.4@0 o.0.8@0")
ORD_EPI2 = os.environ.get("ORD_EPI2", "lp.0.4@0")
ORD_PRO0 = os.environ.get("ORD_PRO0", "v.0.4 f.T.0 f.T.1 q.0.4@0 f.T.2 f.T.3 k.0.1@0 k.1.1@0 k.2.2@0")
LAG = int(os.environ.get("LAG", "2"))
MINI = os.environ.get("MINI", "")
EL = int(os.environ.get("EL", "3"))
NOMAX = int(os.environ.get("NOMAX", "0"))
UNROLL = int(os.environ.get("UNROLL", "1"))

bf16 = jnp.bfloat16
f32 = jnp.float32
u32 = jnp.uint32
i32 = jnp.int32
NT = (((1,), (1,)), ((), ()))


def _al(i, m):
    return i if isinstance(i, int) else pl.multiple_of(i, m)


def _dot(a, b):
    return jnp.dot(a, b, preferred_element_type=f32)


def _dot_nt(a, b):
    return lax.dot_general(a, b, NT, preferred_element_type=f32)


def _phi(t):
    return jnp.where(t > 0, t + 1.0, jnp.exp(t))


def _ln_tiles(xs):
    tot = xs[0]
    for x in xs[1:]:
        tot = tot + x
    mean = jnp.sum(tot, axis=-1, keepdims=True) * (1.0 / D)
    ds = [x - mean for x in xs]
    sq = ds[0] * ds[0]
    for d in ds[1:]:
        sq = sq + d * d
    var = jnp.sum(sq, axis=-1, keepdims=True) * (1.0 / D)
    rstd = lax.rsqrt(var + EPS)
    return [d * rstd for d in ds]


def _kernel(x_hbm, wq_hbm, wk_hbm, wv_hbm, wo_hbm, beta_ref, wr_ref, wg_hbm, wu_hbm, wd_hbm,
            out_hbm, *scr):
    scr = list(scr)

    def take(n):
        out = scr[:n]
        del scr[:n]
        return out
    XIO, X, XN, XB = take(NSEG), take(NSEG), take(NSEG), take(NSEG)
    QS, PQ, KK, PK, VT, OO, ZC = take(2), take(2), take(2), take(2), take(2), take(2), take(2)
    SS = [take(4) for _ in range(4)]
    PP = take(4)
    (WQ, WK, WV, WO, WG, WU, WD, MT, MTB, ZZ, ZB, GATE, ZO, TOP, SEL, WR,
     sem_x, sem_w, sem_f, sem_o, sem_p) = scr

    def x_copy(s, n):
        return pltpu.make_async_copy(
            x_hbm.at[pl.ds(s * L, L), pl.ds(n * 128, 128)], XIO[s].at[n], sem_x.at[s])

    def w_copy(w_hbm, buf, i, n):
        return pltpu.make_async_copy(w_hbm.at[:, pl.ds(_al(n * 128, 128), 128)], buf.at[n], sem_w.at[i, n])

    def f_copy(w_hbm, buf, i, n):
        return pltpu.make_async_copy(w_hbm.at[:, pl.ds(_al(n * 128, 128), 128)], buf.at[n], sem_f.at[i])

    _sc0 = jax.named_scope("s_dmastart"); _sc0.__enter__()
    def start_w(n):
        w_copy(wv_hbm, WV, 2, n).start()
        w_copy(wk_hbm, WK, 1, n).start()
        w_copy(wq_hbm, WQ, 0, n).start()

    for s in range(NSEG):
        for n in range(NG):
            x_copy(s, n).start()
        start_w(2 * s)
        start_w(2 * s + 1)

    _sc0.__exit__(None, None, None)
    def late_copies(g):
        cps = [f_copy(wd_hbm, WD, 2, g)]
        for w_hbm, buf, i in ((wg_hbm, WG, 0), (wu_hbm, WU, 1)):
            for t in range(3):
                cps.append(f_copy(w_hbm, buf, i, g + NG * t))
            r0 = _al((g % 2) * (D // 2), D // 2)
            n = 3 * NG + g // 2
            cps.append(pltpu.make_async_copy(
                w_hbm.at[pl.ds(r0, D // 2), pl.ds(_al(n * 128, 128), 128)],
                buf.at[n, pl.ds(r0, D // 2), :], sem_f.at[i]))
        return cps

    lane = lax.broadcasted_iota(i32, (128, 128), 1)
    row = lax.broadcasted_iota(i32, (128, 128), 0)
    causal = row <= lane
    blockdiag = (row // DH) == (lane // DH)
    lane64 = lax.broadcasted_iota(i32, (64, 128), 1)
    hmask = [jnp.where((lane64 >= h * DH) & (lane64 < (h + 1) * DH), u32(0xFFFFFFFF), u32(0)) for h in range(4)]
    lane8 = lax.broadcasted_iota(i32, (8, 128), 1)
    sub8 = lax.broadcasted_iota(i32, (8, 128), 0)

    _sc1 = jax.named_scope("s_consts"); _sc1.__enter__()
    ZO[0] = 0
    ZO[1] = 0
    gv = jax.nn.sigmoid(beta_ref[...].astype(f32))
    for h in range(H):
        GATE[h] = gv[0, h]

    for n in range(NG):
        WR[n] = jnp.broadcast_to(wr_ref[:, n * 128:(n + 1) * 128].astype(f32), (8, 128))

    _sc1.__exit__(None, None, None)
    def first_ln(t, r0, rows):
        xs = [XIO[t][n, pl.ds(r0, rows), :].astype(f32) for n in range(NG)]
        for n in range(NG):
            X[t][n, pl.ds(r0, rows), :] = xs[n]
        ys = _ln_tiles(xs)
        for n in range(NG):
            XN[t][n, pl.ds(r0, rows), :] = ys[n].astype(bf16)

    def body(s, g, order, has_mem=False, prev=None):
        par = s % 2
        z0, z1 = ZO[0], ZO[1]
        marks = []
        emarks = []
        st = {"m": {}, "mx": {}, "l": {}, "mem": None, "zc": None}
        gates = [GATE[g * 4 + h] for h in range(4)]

        def anchor(lag, *refs):
            lag = min(lag, len(marks))
            if lag == 0:
                return
            mk = marks[-lag]
            for ref in refs:
                slot = ref.shape[0] - 1
                if ref.dtype == f32:
                    val = mk
                else:
                    val = jnp.concatenate([mk, mk], axis=0).astype(ref.dtype)
                idx = (slot + z0,) + (0,) * (len(ref.shape) - 3) + (pl.ds(_al(z0 * val.shape[0], val.shape[0]), val.shape[0]), slice(None))
                ref[idx] = val

        def xn_lhs(t, c, nc):
            return jnp.concatenate([XN[t][k, pl.ds(c * 128, nc * 128), :] for k in range(NG)], axis=1)

        def q_proj(lag, c, nc=1):
            t, tp = s + 1, 1 - par
            anchor(lag, XN[t], WQ)
            q = _dot(xn_lhs(t, c, nc), WQ[g])
            marks.append(q[0:8])
            rows = pl.ds(c * 128, nc * 128)
            QS[tp][g, rows, :] = (q * QSCALE).astype(bf16)
            PQ[tp][g, rows, :] = _phi(q).astype(bf16)

        def k_proj(lag, c, nc=1):
            t, tp = s + 1, 1 - par
            anchor(lag, XN[t], WK)
            k = _dot(xn_lhs(t, c, nc), WK[g])
            marks.append(k[0:8])
            rows = pl.ds(c * 128, nc * 128)
            KK[tp][g, rows, :] = k.astype(bf16)
            pk = _phi(k)
            PK[tp][g, rows, :] = pk.astype(bf16)
            zc = st["zc"]
            for r in range(nc * 16):
                zc = pk[r * 8:(r + 1) * 8] if zc is None else zc + pk[r * 8:(r + 1) * 8]
            st["zc"] = zc
            if c + nc == 4:
                ZC[tp][g] = zc

        def v_proj(lag, c, nc=1):
            t, tp = s + 1, 1 - par
            anchor(lag, XN[t], WV)
            v = _dot(xn_lhs(t, c, nc), WV[g])
            marks.append(v[0:8])
            v = v.astype(bf16)
            for j in range(nc):
                VT[tp][g, c + j] = v[j * 128:(j + 1) * 128, :].T

        def o_proj(lag, n0, nn=2):
            t, tp = s - 1, 1 - par
            cr = _al(g * CH, CH)
            anchor(lag, OO[tp], WO)
            lhs = jnp.concatenate([OO[tp][k, pl.ds(cr, CH), :] for k in range(NG)], axis=1)
            rhs = jnp.concatenate([WO[n] for n in range(n0, n0 + nn)], axis=1)
            att = _dot(lhs, rhs)
            marks.append(att[0:8, 0:128])
            for i in range(nn):
                n = n0 + i
                X[t][n + z0, pl.ds(cr, CH), :] = X[t][n, pl.ds(cr, CH), :] + att[:, i * 128:(i + 1) * 128]

        def o_lp(lag, c, nc=1):
            if prev is not None:
                o_ln(lag, c, nc, *prev)

        def o_ln(lag, c, nc=1, t=s - 1, g=g):
            anchor(lag, X[t])
            R = 16 * nc
            r0 = _al(g * CH + c * 16, 16)
            x1 = [X[t][n + z1, pl.ds(r0, R), :] for n in range(NG)]
            xb = _ln_tiles(x1)
            wr = [jnp.concatenate([WR[n]] * (R // 8), axis=0) for n in range(NG)]
            acc = xb[0] * wr[0]
            for n in range(1, NG):
                acc = acc + xb[n] * wr[n]
            r = jnp.broadcast_to(jnp.sum(acc, axis=-1, keepdims=True), (R, 128))
            m1, i1, m2, i2 = TOP[0], TOP[1], TOP[2], TOP[3]
            for u in range(R // 8):
                rv = r[u * 8:(u + 1) * 8, :]
                iv = (sub8 + (r0 + (t * L + u * 8))).astype(f32)
                g1 = rv > m1
                g2 = rv > m2
                m2 = jnp.where(g1, m1, jnp.where(g2, rv, m2))
                i2 = jnp.where(g1, i1, jnp.where(g2, iv, i2))
                m1 = jnp.where(g1, rv, m1)
                i1 = jnp.where(g1, iv, i1)
            TOP[0] = m1
            TOP[1] = i1
            TOP[2] = m2
            TOP[3] = i2
            x2 = [x1[n] + xb[n] for n in range(NG)]
            for n in range(NG):
                X[t][n, pl.ds(r0, R), :] = x2[n]
                XB[t][n, pl.ds(r0, R), :] = xb[n].astype(bf16)
                XIO[t][n, pl.ds(r0, R), :] = x2[n].astype(bf16)
            xn = _ln_tiles(x2)
            for n in range(NG):
                XN[t][n, pl.ds(r0, R), :] = xn[n].astype(bf16)

        def qk(lag, i):
            nk = (i + 1) * 128
            anchor(lag, QS[par], KK[par])
            qu = pltpu.bitcast(QS[par][g, pl.ds(i * 128, 128), :], u32)
            qm = jnp.concatenate([pltpu.bitcast(qu & hmask[h], bf16) for h in range(4)], axis=0)
            sT = _dot_nt(KK[par][g, pl.ds(0, nk), :], qm)
            marks.append(sT[0:8, 0:128])
            if NOMAX:
                for h in range(4):
                    l = None
                    for r in range(nk // 16):
                        t = sT[r * 16:(r + 1) * 16, h * 128:(h + 1) * 128]
                        if r >= i * 8:
                            t = jnp.where(causal[(r - i * 8) * 16:(r - i * 8 + 1) * 16], t, NEG)
                        e = jnp.exp2(t)
                        es = e[0:8] + e[8:16]
                        l = es if l is None else l + es
                        PP[i][h + z0, pl.ds(r * 16, 16), :] = e.astype(bf16)
                    st["l"][(i, h)] = jnp.sum(l, axis=0, keepdims=True)
                return
            for h in range(4):
                mx = None
                for r in range(nk // 8):
                    t = sT[r * 8:(r + 1) * 8, h * 128:(h + 1) * 128]
                    if r >= i * 16:
                        t = jnp.where(causal[(r - i * 16) * 8:(r - i * 16 + 1) * 8], t, NEG)
                    mx = t if mx is None else jnp.maximum(mx, t)
                    SS[i][h][z0, pl.ds(r * 8, 8), :] = t
                st["m"][(i, h)] = jnp.max(mx, axis=0, keepdims=True)

        def sm(lag, i, h0, nh=1):
            if NOMAX:
                return
            for h in range(h0, h0 + nh):
                m = st["m"][(i, h)]
                la = [None, None]
                for j in range(i + 1):
                    if len(emarks) >= EL:
                        SS[i][h][1 + z0, pl.ds(_al(z0 * 8, 8), 8), :] = emarks[-EL]
                    else:
                        anchor(lag, SS[i][h])
                    for r in range(j * 8, (j + 1) * 8):
                        e = jnp.exp2(SS[i][h][z1, pl.ds(r * 16, 16), :] - m)
                        es = e[0:8] + e[8:16]
                        la[r % 2] = es if la[r % 2] is None else la[r % 2] + es
                        PP[i][h + z0, pl.ds(r * 16, 16), :] = e.astype(bf16)
                    emarks.append(la[0] + la[1])
                st["l"][(i, h)] = jnp.sum(la[0] + la[1], axis=0, keepdims=True)

        def qs(lag, i, j):
            anchor(lag, QS[par], KK[par])
            qu = pltpu.bitcast(QS[par][g, pl.ds(i * 128, 128), :], u32)
            qm = jnp.concatenate([pltpu.bitcast(qu & hmask[h], bf16) for h in range(4)], axis=0)
            sT = _dot_nt(KK[par][g, pl.ds(j * 128, 128), :], qm)
            marks.append(sT[0:8, 0:128])
            done = st.setdefault("nq", {}).get(i, 0) + 1
            st["nq"][i] = done
            for h in range(4):
                mx = st["mx"].get((i, h))
                for r in range(16):
                    t = sT[r * 8:(r + 1) * 8, h * 128:(h + 1) * 128]
                    if j == i:
                        t = jnp.where(causal[r * 8:(r + 1) * 8], t, NEG)
                    mx = t if mx is None else jnp.maximum(mx, t)
                    SS[i][h][z0, pl.ds(j * 128 + r * 8, 8), :] = t
                st["mx"][(i, h)] = mx
                if done == i + 1:
                    st["m"][(i, h)] = jnp.max(mx, axis=0, keepdims=True)

        def ps(lag, i, j):
            anchor(lag, *SS[i], VT[par])
            done = st.setdefault("np", {}).get(i, 0) + 1
            st["np"][i] = done
            outs = []
            for h in range(4):
                m = st["m"][(i, h)]
                la = st.setdefault("la", {}).setdefault((i, h), [None, None])
                packed = []
                for r in range(8):
                    e = jnp.exp2(SS[i][h][z1, pl.ds(j * 128 + r * 16, 16), :] - m)
                    es = e[0:8] + e[8:16]
                    la[r % 2] = es if la[r % 2] is None else la[r % 2] + es
                    packed.append(e.astype(bf16))
                o = _dot(VT[par][g, j, pl.ds(h * DH, DH), :], jnp.concatenate(packed, axis=0))
                if h == 0:
                    marks.append(o[0:8])
                acc = st.setdefault("acc", {}).get((i, h))
                acc = o if acc is None else acc + o
                st["acc"][(i, h)] = acc
                if done == i + 1:
                    l = jnp.sum(la[0] + la[1], axis=0, keepdims=True)
                    outs.append(finish(i, h, acc, l))
            if done == i + 1:
                OO[par][g, pl.ds(i * 128, 128), :] = jnp.concatenate(outs, axis=0).astype(bf16).T

        def finish(i, h, oT, l):
            o = oT * ((1.0 - gates[h]) / l)
            if has_mem:
                memT = st["mem"]
                num = memT[h * DH:(h + 1) * DH, i * 128:(i + 1) * 128]
                den = memT[128 + h * 8:128 + (h + 1) * 8, i * 128:(i + 1) * 128] + 1e-6
                w = gates[h] / den
                o = o + num * jnp.concatenate([w] * 4, axis=0)
            return o

        def mem(lag):
            anchor(lag, MTB, PQ[par])
            lhs = jnp.concatenate([MTB[g], ZB[g]], axis=0)
            st["mem"] = _dot_nt(lhs, PQ[par][g])
            marks.append(st["mem"][0:8, 0:128])

        def pv(lag, i):
            nk = (i + 1) * 128
            anchor(lag, VT[par], PP[i])
            outs = []
            for h in range(4):
                vt = jnp.concatenate([VT[par][g, j, pl.ds(h * DH, DH), :] for j in range(i + 1)], axis=1)
                oT = _dot(vt, PP[i][h + z1])
                if h == 0:
                    marks.append(oT[0:8])
                outs.append(finish(i, h, oT, st["l"][(i, h)]))
            oT_all = jnp.concatenate(outs, axis=0).astype(bf16)
            OO[par][g, pl.ds(i * 128, 128), :] = oT_all.T

        def upd(lag):
            anchor(lag, VT[par], PK[par])
            vt_all = jnp.concatenate([VT[par][g, j] for j in range(4)], axis=1)
            dm = _dot(vt_all, PK[par][g])
            marks.append(dm[0:8])
            mt = MT[g] + jnp.where(blockdiag, dm, 0.0)
            MT[g] = mt
            MTB[g] = mt.astype(bf16)
            z = ZZ[g] + jnp.sum(ZC[par][g], axis=0, keepdims=True)
            ZZ[g] = z
            ZB[g] = jnp.concatenate(
                [jnp.where((lane8 >= h * DH) & (lane8 < (h + 1) * DH), z, 0.0) for h in range(4)], axis=0).astype(bf16)

        def fln(lag, t, c):
            first_ln(t, _al((g - 2 * t) * 256 + c * 64, 64), 64)

        table = {"qs": qs, "ps": ps, "lp": o_lp, "f": fln, "qk": qk, "sm": sm, "pv": pv, "mem": mem, "upd": upd,
                 "o": o_proj, "ln": o_ln, "q": q_proj, "k": k_proj, "v": v_proj}
        for kind, args, lag in order:
            table[kind](lag, *args)

    def parse(txt, drop=()):
        out = []
        for w in txt.split():
            lag = LAG
            if "@" in w:
                w, lg = w.split("@")
                lag = int(lg)
            p = w.split(".")
            if p[0] not in drop:
                out.append((p[0], tuple(int(x) for x in p[1:]), lag))
        return out

    FULL = parse(ORD_FULL)
    FIRST = parse(ORD_FIRST)
    LAST = parse(ORD_LAST)
    PRO = parse(ORD_PRO)
    EPI = parse(ORD_EPI)
    EPI2 = parse(ORD_EPI2)

    if MINI:
        order, hm, sg = {"full": (FULL, True, 1), "first": (FIRST, False, 0), "last": (LAST, True, 3),
                         "pro": (PRO, False, -1), "epi": (EPI, False, 4)}[MINI]

        def b(g, c):
            body(sg, g, order, hm, (sg - 1, g - 1) if MINI == "last" else None)
            return c
        lax.fori_loop(1 if MINI == "last" else 0, NG, b, 0)
        return

    with jax.named_scope("s_xwait0"):
        for n in range(NG):
            x_copy(0, n).wait()

    def ln0(c, carry):
        first_ln(0, _al(c * CH, CH), CH)
        return carry
    with jax.named_scope("s_ln0"):
        lax.fori_loop(0, NG, ln0, 0)

    for t in range(NSEG):
        if t > 0:
          with jax.named_scope(f"s_xwait{t}"):
            for n in range(NG):
                x_copy(t, n).wait()

        if t == 2:
            for n in range(NG):
                w_copy(wo_hbm, WO, 3, n).start()

        def pro0(g, c, t=t):
            for i, w in ((2, WV), (1, WK), (0, WQ)):
                pltpu.make_async_copy(w.at[g], w.at[g], sem_w.at[i, g]).wait()
            body(-1, g, PRO if t == 0 else parse(ORD_PRO0.replace("T", str(t))))
            return c
        with jax.named_scope(f"s_pro0_{t}"):
            lax.fori_loop(2 * t, 2 * t + 2, pro0, 0)

    for n in range(NG):
        w_copy(wo_hbm, WO, 3, n).wait()

    def layer(li, carry):
        _sc2 = jax.named_scope("s_reset"); _sc2.__enter__()
        MT[...] = jnp.zeros(MT.shape, f32)
        ZZ[...] = jnp.zeros(ZZ.shape, f32)
        TOP[0] = jnp.full((8, 128), -jnp.inf, f32)
        TOP[1] = jnp.zeros((8, 128), f32)
        TOP[2] = jnp.full((8, 128), -jnp.inf, f32)
        TOP[3] = jnp.zeros((8, 128), f32)

        _sc2.__exit__(None, None, None)
        def out_copy(s, n):
            return pltpu.make_async_copy(
                XIO[s].at[n], out_hbm.at[pl.ds(s * L, L), pl.ds(n * 128, 128)], sem_o.at[0])

        def loop(s, order, has_mem, extra=None):
            def b(g, c):
                for u in range(UNROLL):
                    if extra is not None:
                        extra(g * UNROLL + u)
                    body(s, g * UNROLL + u, order, has_mem)
                return c
            with jax.named_scope(f"s_loop{s}"):
                lax.fori_loop(0, NG // UNROLL, b, 0)

        def start_late(g):
            for cp in late_copies(g):
                cp.start()

        def flush(s):
            @pl.when(li == 1)
            def _():
                for n in range(NG):
                    out_copy(s, n).start()

        loop(0, FIRST, False, start_late)
        loop(1, FULL, True)
        loop(2, FULL, True)
        flush(0)
        body(3, 0, LAST, True)

        def b3(g, c):
            body(3, g, LAST, True, (2, g - 1))
            return c
        with jax.named_scope("s_loop3"):
            lax.fori_loop(1, NG, b3, 0)
        flush(1)
        with jax.named_scope("s_epi"):
            for c in range(NG + 1):
                body(4, c, EPI if c < NG else EPI2, False, (2, NG - 1) if c == 0 else (3, c - 1))
        flush(2)
        flush(3)

        _sc = jax.named_scope('s_top2'); _sc.__enter__()
        m1, i1, m2, i2 = TOP[0], TOP[1], TOP[2], TOP[3]
        big = f32(1e9)
        ra = jnp.max(m1, axis=0, keepdims=True)
        ia = jnp.min(jnp.where(m1 == ra, i1, big), axis=0, keepdims=True)
        isa = i1 == ia
        cv = jnp.where(isa, m2, m1)
        ci = jnp.where(isa, i2, i1)
        rb = jnp.max(cv, axis=0, keepdims=True)
        ib = jnp.min(jnp.where(cv == rb, ci, big), axis=0, keepdims=True)
        idx = [ia.astype(i32)[0, 0], ib.astype(i32)[0, 0]]
        idx = [jnp.clip(t, 0, S - 1) for t in idx]
        row16 = lax.broadcasted_iota(i32, (16, 128), 0)
        gsel = jnp.where(row16 == 0, jax.nn.sigmoid(ra), jnp.where(row16 == 1, jax.nn.sigmoid(rb), 0.0))

        seg = [t // L for t in idx]
        loc = [t % L for t in idx]
        base = [pl.multiple_of((t // 16) * 16, 16) for t in loc]
        off = [t % 16 for t in loc]
        for t in range(2):
            for s in range(NSEG):
                @pl.when(seg[t] == s)
                def _(t=t, s=s):
                    for n in range(NG):
                        blk = XB[s][n, pl.ds(base[t], 16), :].astype(f32)
                        SEL[t, n] = jnp.broadcast_to(
                            jnp.sum(jnp.where(row16 == off[t], blk, 0.0), axis=0, keepdims=True), (8, 128))
        xsel = []
        for n in range(NG):
            r0_ = SEL[0, n][0:1]
            r1_ = SEL[1, n][0:1]
            xsel.append(jnp.where(row16 == 0, r0_, jnp.where(row16 == 1, r1_, 0.0)))
        xsel = jnp.concatenate(xsel, axis=1).astype(bf16)

        _sc.__exit__(None, None, None)
        _sc = jax.named_scope('s_ffn'); _sc.__enter__()
        pltpu.make_async_copy(WG, WG, sem_f.at[0]).wait()
        pltpu.make_async_copy(WU, WU, sem_f.at[1]).wait()
        pltpu.make_async_copy(WD, WD, sem_f.at[2]).wait()

        wg = jnp.concatenate([WG[n] for n in range(NF)], axis=1)
        wu = jnp.concatenate([WU[n] for n in range(NF)], axis=1)
        gg = _dot(xsel, wg)
        uu = _dot(xsel, wu)
        hh = (gg * jax.nn.sigmoid(gg) * uu).astype(bf16)
        wd = jnp.concatenate([WD[n] for n in range(NG)], axis=1)
        y = _dot(hh, wd)

        _sc.__exit__(None, None, None)
        _sc = jax.named_scope('s_fix'); _sc.__enter__()
        @pl.when(li == 1)
        def _():
            for s in range(NSEG):
                for n in range(NG):
                    out_copy(s, n).wait()

        for t in range(2):
            b8 = pl.multiple_of((loc[t] // 8) * 8, 8)
            o8 = loc[t] % 8
            yrows = []
            for n in range(NG):
                yt = y[:, n * 128:(n + 1) * 128] * gsel
                yrows.append(jnp.sum(jnp.where(row16 == t, yt, 0.0), axis=0, keepdims=True))
            for s in range(NSEG):
                @pl.when(seg[t] == s)
                def _(t=t, s=s, b8=b8, o8=o8, yrows=yrows):
                    xs = []
                    for n in range(NG):
                        blk = X[s][n, pl.ds(b8, 8), :]
                        blk = jnp.where(sub8 == o8, blk + yrows[n], blk)
                        X[s][n, pl.ds(b8, 8), :] = blk
                        xs.append(blk)
                    xn = _ln_tiles(xs)
                    sel = row16 == off[t]
                    for n in range(NG):
                        new_x = jnp.sum(jnp.where(sub8 == o8, xs[n], 0.0), axis=0, keepdims=True)
                        new_n = jnp.sum(jnp.where(sub8 == o8, xn[n], 0.0), axis=0, keepdims=True)
                        blk = XN[s][n, pl.ds(base[t], 16), :]
                        XN[s][n, pl.ds(base[t], 16), :] = jnp.where(sel, new_n, blk.astype(f32)).astype(bf16)
                        blk = XIO[s][n, pl.ds(base[t], 16), :]
                        XIO[s][n, pl.ds(base[t], 16), :] = jnp.where(sel, new_x, blk.astype(f32)).astype(bf16)

                    @pl.when(li == 1)
                    def _():
                        cps = [pltpu.make_async_copy(
                            XIO[s].at[n, pl.ds(base[t], 16), :],
                            out_hbm.at[pl.ds(s * L + base[t], 16), pl.ds(n * 128, 128)], sem_p.at[0])
                            for n in range(NG)]
                        for cp in cps:
                            cp.start()
                        for cp in cps:
                            cp.wait()
        _sc.__exit__(None, None, None)

        @pl.when(li == 0)
        def _():
            def pro(g, c):
                body(-1, g, PRO)
                return c
            with jax.named_scope("s_pro"):
                lax.fori_loop(0, NG, pro, 0)
        return carry

    lax.fori_loop(0, 2, layer, 0)


def _build(interpret=False):
    any_spec = pl.BlockSpec(memory_space=pl.ANY)
    vmem_spec = pl.BlockSpec(memory_space=pltpu.VMEM)
    V = pltpu.VMEM
    A = NG + 1
    scratch = (
        [V((NG, L, 128), bf16)] * NSEG + [V((A, L, 128), f32)] * NSEG
        + [V((A, L, 128), bf16)] * NSEG + [V((NG, L, 128), bf16)] * NSEG
        + [V((A, L, 128), bf16)] * 8
        + [V((A, 4, 128, 128), bf16)] * 2
        + [V((A, L, 128), bf16)] * 2
        + [V((NG, 8, 128), f32)] * 2
        + [V((2, (i + 1) * 128, 128), f32) for i in range(4) for _ in range(4)]
        + [V((5, (i + 1) * 128, 128), bf16) for i in range(4)]
    ) + [
        V((A, D, 128), bf16), V((A, D, 128), bf16), V((A, D, 128), bf16), V((A, D, 128), bf16),
        V((NF, D, 128), bf16), V((NF, D, 128), bf16), V((NG, F, 128), bf16),
        V((NG, 128, 128), f32), V((A, 128, 128), bf16),
        V((NG, 8, 128), f32), V((NG, 32, 128), bf16),
        pltpu.SMEM((H,), f32),
        pltpu.SMEM((2,), i32),
        V((4, 8, 128), f32),
        V((2, NG, 8, 128), f32),
        V((NG, 8, 128), f32),
        pltpu.SemaphoreType.DMA((NSEG,)),
        pltpu.SemaphoreType.DMA((4, NG)),
        pltpu.SemaphoreType.DMA((3,)),
        pltpu.SemaphoreType.DMA((1,)),
        pltpu.SemaphoreType.DMA((1,)),
    ]
    return pl.pallas_call(
        _kernel,
        out_shape=jax.ShapeDtypeStruct((S, D), bf16),
        in_specs=[any_spec] * 5 + [vmem_spec, vmem_spec] + [any_spec] * 3,
        out_specs=any_spec,
        scratch_shapes=scratch,
        compiler_params=pltpu.CompilerParams(vmem_limit_bytes=110 * 1024 * 1024, flags=(__import__("json").loads(os.environ.get("KFLAGS", "{}")) or None)),
        interpret=pltpu.InterpretParams() if interpret else False,
        name="infini_mod",
    )


@jax.jit
def pallas_interleave_layers__memory_aug_infini_attn__moe_arch_mod__prompt_kernel(
    A_x, A_wq, A_wk, A_wv, A_wo, A_beta, B_x, B_w_r, B_w_gate, B_w_up, B_w_down,
):
    del B_x
    out = _build()(A_x.reshape(S, D), A_wq, A_wk, A_wv, A_wo, A_beta.reshape(1, H), B_w_r.reshape(1, D),
                   B_w_gate, B_w_up, B_w_down)
    return out.reshape(1, S, D)
```

```python
import jax
import jax.numpy as jnp
from jax import lax
import jax.experimental.pallas as pl
import jax.experimental.pallas.tpu as pltpu

S = 2048
D = 1024
NSEG = 4
L = S // NSEG
H = 32
DH = D // H
NG = 8
F = 3584
NF = F // 128
CH = L // NG
EPS = 1e-5
LOG2E = 1.4426950408889634
QSCALE = (DH ** -0.5) * LOG2E
NEG = -1e30

ORD_FULL = "o.0.8@0 qk.3@3 qk.0@0 ln.0.1@3 k.0.4 ln.1.1@1 qk.2@0 sm.3.2.2@0 ln.2.2@0 mem@2 qk.1@2 sm.3.0.2@2 v.0.4 pv.3@0 sm.2.2.2@2 sm.2.0.1@2 sm.2.1.1@2 sm.1.0.4@0 pv.2 sm.0.0.4@1 pv.1@2 pv.0@3 q.0.4@0 upd"
ORD_FIRST = "qk.2@2 k.0.4@0 qk.1@3 sm.2.1.3@0 sm.1.0.1@0 v.0.1@0 sm.2.0.1@3 sm.1.1.1@0 qk.3@2 sm.1.2.2@0 q.0.2@0 sm.3.0.4@1 upd@0 qk.0@2 v.3.1@0 sm.0.2.2@3 v.2.1@0 sm.0.0.2@0 v.1.1@3 pv.3@0 pv.0@3 pv.2@3 pv.1@0 q.2.2@0"
ORD_LAST = "qk.2@2 qk.3@2 sm.2.0.1@2 sm.2.2.2@2 sm.2.1.1@2 qk.1@1 sm.3.0.4@2 lp.0.4@3 sm.1.1.1@0 mem@0 sm.1.0.1@3 o.0.4@0 sm.1.3.1@0 qk.0@2 sm.1.2.1@0 pv.2 sm.0.0.4@0 pv.3@3 pv.1@0 pv.0@2 o.4.4@0"
ORD_START = "g.0 g.1 x.1 x.2 x.3 w.2 w.0 w.1 v.0.1@0 g.2 g.3 v.1.1@0 g.4 g.5 v.2.1@0 g.6 g.7 v.3.1@0 q.0.4@0 k.0.1@0 k.1.1@0 k.2.2@0"
ORD_PRO = "v.0.4 q.0.4@0 k.0.1@0 k.1.1@0 k.2.2@0"
ORD_EPI = "lp.0.4@0 o.0.8@0"
ORD_EPI2 = "lp.0.4@0"
ORD_PRO0 = "v.0.4 f.T.0 f.T.1 q.0.4@0 f.T.2 f.T.3 k.0.1@0 k.1.1@0 k.2.2@0"
LAG = 2
EL = 3

bf16 = jnp.bfloat16
f32 = jnp.float32
u32 = jnp.uint32
i32 = jnp.int32
NT = (((1,), (1,)), ((), ()))


def _al(i, m):
    return i if isinstance(i, int) else pl.multiple_of(i, m)


def _dot(a, b):
    return jnp.dot(a, b, preferred_element_type=f32)


def _dot_nt(a, b):
    return lax.dot_general(a, b, NT, preferred_element_type=f32)


def _phi(t):
    return jnp.where(t > 0, t + 1.0, jnp.exp(t))


def _ln_tiles(xs):
    tot = xs[0]
    for x in xs[1:]:
        tot = tot + x
    mean = jnp.sum(tot, axis=-1, keepdims=True) * (1.0 / D)
    ds = [x - mean for x in xs]
    sq = ds[0] * ds[0]
    for d in ds[1:]:
        sq = sq + d * d
    var = jnp.sum(sq, axis=-1, keepdims=True) * (1.0 / D)
    rstd = lax.rsqrt(var + EPS)
    return [d * rstd for d in ds]


def _kernel(x_hbm, wq_hbm, wk_hbm, wv_hbm, wo_hbm, beta_ref, wr_ref, wg_hbm, wu_hbm, wd_hbm,
            out_hbm, *scr):
    scr = list(scr)

    def take(n):
        out = scr[:n]
        del scr[:n]
        return out
    XIO, X, XN, XB = take(NSEG), take(NSEG), take(NSEG), take(NSEG)
    QS, PQ, KK, PK, VT, OO, ZC = take(2), take(2), take(2), take(2), take(2), take(2), take(2)
    SS = [take(4) for _ in range(4)]
    PP = take(4)
    (WQ, WK, WV, WO, WG, WU, WD, MT, MTB, ZZ, ZB, GATE, ZO, TOP, SEL, WR, X0,
     sem_0, sem_x, sem_w, sem_f, sem_o, sem_p) = scr

    def x_copy(s, n):
        return pltpu.make_async_copy(
            x_hbm.at[pl.ds(s * L, L), pl.ds(n * 128, 128)], XIO[s].at[n], sem_x.at[s])

    def w_copy(w_hbm, buf, i, n):
        return pltpu.make_async_copy(w_hbm.at[:, pl.ds(_al(n * 128, 128), 128)], buf.at[n], sem_w.at[i, n])

    def f_copy(w_hbm, buf, i, n):
        return pltpu.make_async_copy(w_hbm.at[:, pl.ds(_al(n * 128, 128), 128)], buf.at[n], sem_f.at[i])
    def start_w(n):
        w_copy(wv_hbm, WV, 2, n).start()
        w_copy(wk_hbm, WK, 1, n).start()
        w_copy(wq_hbm, WQ, 0, n).start()

    def x0_copy(c):
        rows = pl.ds(c * 128, 128)
        return pltpu.make_async_copy(x_hbm.at[rows, :], X0.at[rows, :], sem_0.at[c])

    for c in range(4):
        x0_copy(c).start()
    start_w(0)

    def start_rest():
        start_w(1)
        for s in range(1, NSEG):
            for n in range(NG):
                x_copy(s, n).start()
            start_w(2 * s)
            start_w(2 * s + 1)
    def late_copies(g):
        cps = [f_copy(wd_hbm, WD, 2, g)]
        for w_hbm, buf, i in ((wg_hbm, WG, 0), (wu_hbm, WU, 1)):
            for t in range(3):
                cps.append(f_copy(w_hbm, buf, i, g + NG * t))
            r0 = _al((g % 2) * (D // 2), D // 2)
            n = 3 * NG + g // 2
            cps.append(pltpu.make_async_copy(
                w_hbm.at[pl.ds(r0, D // 2), pl.ds(_al(n * 128, 128), 128)],
                buf.at[n, pl.ds(r0, D // 2), :], sem_f.at[i]))
        return cps

    lane = lax.broadcasted_iota(i32, (128, 128), 1)
    row = lax.broadcasted_iota(i32, (128, 128), 0)
    causal = row <= lane
    blockdiag = (row // DH) == (lane // DH)
    lane64 = lax.broadcasted_iota(i32, (64, 128), 1)
    hmask = [jnp.where((lane64 >= h * DH) & (lane64 < (h + 1) * DH), u32(0xFFFFFFFF), u32(0)) for h in range(4)]
    lane8 = lax.broadcasted_iota(i32, (8, 128), 1)
    sub8 = lax.broadcasted_iota(i32, (8, 128), 0)
    ZO[0] = 0
    ZO[1] = 0
    gv = jax.nn.sigmoid(beta_ref[...].astype(f32))
    for h in range(H):
        GATE[h] = gv[0, h]

    for n in range(NG):
        WR[n] = jnp.broadcast_to(wr_ref[n:n + 1, :].astype(f32), (8, 128))
    def first_ln(t, r0, rows):
        xs = [XIO[t][n, pl.ds(r0, rows), :].astype(f32) for n in range(NG)]
        for n in range(NG):
            X[t][n, pl.ds(r0, rows), :] = xs[n]
        ys = _ln_tiles(xs)
        for n in range(NG):
            XN[t][n, pl.ds(r0, rows), :] = ys[n].astype(bf16)

    def body(s, g, order, has_mem=False, prev=None):
        par = s % 2
        z0, z1 = ZO[0], ZO[1]
        marks = []
        emarks = []
        st = {"m": {}, "mx": {}, "l": {}, "mem": None, "zc": None}
        gates = [GATE[g * 4 + h] for h in range(4)]

        def anchor(lag, *refs):
            lag = min(lag, len(marks))
            if lag == 0:
                return
            mk = marks[-lag]
            for ref in refs:
                slot = ref.shape[0] - 1
                if ref.dtype == f32:
                    val = mk
                else:
                    val = jnp.concatenate([mk, mk], axis=0).astype(ref.dtype)
                idx = (slot + z0,) + (0,) * (len(ref.shape) - 3) + (pl.ds(_al(z0 * val.shape[0], val.shape[0]), val.shape[0]), slice(None))
                ref[idx] = val

        def xn_lhs(t, c, nc):
            return jnp.concatenate([XN[t][k, pl.ds(c * 128, nc * 128), :] for k in range(NG)], axis=1)

        def q_proj(lag, c, nc=1):
            t, tp = s + 1, 1 - par
            anchor(lag, XN[t], WQ)
            q = _dot(xn_lhs(t, c, nc), WQ[g])
            marks.append(q[0:8])
            rows = pl.ds(c * 128, nc * 128)
            QS[tp][g, rows, :] = (q * QSCALE).astype(bf16)
            PQ[tp][g, rows, :] = _phi(q).astype(bf16)

        def k_proj(lag, c, nc=1):
            t, tp = s + 1, 1 - par
            anchor(lag, XN[t], WK)
            k = _dot(xn_lhs(t, c, nc), WK[g])
            marks.append(k[0:8])
            rows = pl.ds(c * 128, nc * 128)
            KK[tp][g, rows, :] = k.astype(bf16)
            pk = _phi(k)
            PK[tp][g, rows, :] = pk.astype(bf16)
            zc = st["zc"]
            for r in range(nc * 16):
                zc = pk[r * 8:(r + 1) * 8] if zc is None else zc + pk[r * 8:(r + 1) * 8]
            st["zc"] = zc
            if c + nc == 4:
                ZC[tp][g] = zc

        def v_proj(lag, c, nc=1):
            t, tp = s + 1, 1 - par
            anchor(lag, XN[t], WV)
            v = _dot(xn_lhs(t, c, nc), WV[g])
            marks.append(v[0:8])
            v = v.astype(bf16)
            for j in range(nc):
                VT[tp][g, c + j] = v[j * 128:(j + 1) * 128, :].T

        def o_proj(lag, n0, nn=2):
            t, tp = s - 1, 1 - par
            cr = _al(g * CH, CH)
            anchor(lag, OO[tp], WO)
            lhs = jnp.concatenate([OO[tp][k, pl.ds(cr, CH), :] for k in range(NG)], axis=1)
            rhs = jnp.concatenate([WO[n] for n in range(n0, n0 + nn)], axis=1)
            att = _dot(lhs, rhs)
            marks.append(att[0:8, 0:128])
            for i in range(nn):
                n = n0 + i
                X[t][n + z0, pl.ds(cr, CH), :] = X[t][n, pl.ds(cr, CH), :] + att[:, i * 128:(i + 1) * 128]

        def o_lp(lag, c, nc=1):
            if prev is not None:
                o_ln(lag, c, nc, *prev)

        def o_ln(lag, c, nc=1, t=s - 1, g=g):
            anchor(lag, X[t])
            R = 16 * nc
            r0 = _al(g * CH + c * 16, 16)
            x1 = [X[t][n + z1, pl.ds(r0, R), :] for n in range(NG)]
            xb = _ln_tiles(x1)
            wr = [jnp.concatenate([WR[n]] * (R // 8), axis=0) for n in range(NG)]
            acc = xb[0] * wr[0]
            for n in range(1, NG):
                acc = acc + xb[n] * wr[n]
            r = jnp.broadcast_to(jnp.sum(acc, axis=-1, keepdims=True), (R, 128))
            m1, i1, m2, i2 = TOP[0], TOP[1], TOP[2], TOP[3]
            for u in range(R // 8):
                rv = r[u * 8:(u + 1) * 8, :]
                iv = (sub8 + (r0 + (t * L + u * 8))).astype(f32)
                g1 = rv > m1
                g2 = rv > m2
                m2 = jnp.where(g1, m1, jnp.where(g2, rv, m2))
                i2 = jnp.where(g1, i1, jnp.where(g2, iv, i2))
                m1 = jnp.where(g1, rv, m1)
                i1 = jnp.where(g1, iv, i1)
            TOP[0] = m1
            TOP[1] = i1
            TOP[2] = m2
            TOP[3] = i2
            x2 = [x1[n] + xb[n] for n in range(NG)]
            for n in range(NG):
                X[t][n, pl.ds(r0, R), :] = x2[n]
                XB[t][n, pl.ds(r0, R), :] = xb[n].astype(bf16)
                XIO[t][n, pl.ds(r0, R), :] = x2[n].astype(bf16)
            xn = _ln_tiles(x2)
            for n in range(NG):
                XN[t][n, pl.ds(r0, R), :] = xn[n].astype(bf16)

        def qk(lag, i):
            nk = (i + 1) * 128
            anchor(lag, QS[par], KK[par])
            qu = pltpu.bitcast(QS[par][g, pl.ds(i * 128, 128), :], u32)
            qm = jnp.concatenate([pltpu.bitcast(qu & hmask[h], bf16) for h in range(4)], axis=0)
            sT = _dot_nt(KK[par][g, pl.ds(0, nk), :], qm)
            marks.append(sT[0:8, 0:128])
            for h in range(4):
                mx = None
                for r in range(nk // 8):
                    t = sT[r * 8:(r + 1) * 8, h * 128:(h + 1) * 128]
                    if r >= i * 16:
                        t = jnp.where(causal[(r - i * 16) * 8:(r - i * 16 + 1) * 8], t, NEG)
                    mx = t if mx is None else jnp.maximum(mx, t)
                    SS[i][h][z0, pl.ds(r * 8, 8), :] = t
                st["m"][(i, h)] = jnp.max(mx, axis=0, keepdims=True)

        def sm(lag, i, h0, nh=1):
            for h in range(h0, h0 + nh):
                m = st["m"][(i, h)]
                la = [None, None]
                for j in range(i + 1):
                    if len(emarks) >= EL:
                        SS[i][h][1 + z0, pl.ds(_al(z0 * 8, 8), 8), :] = emarks[-EL]
                    else:
                        anchor(lag, SS[i][h])
                    for r in range(j * 8, (j + 1) * 8):
                        e = jnp.exp2(SS[i][h][z1, pl.ds(r * 16, 16), :] - m)
                        es = e[0:8] + e[8:16]
                        la[r % 2] = es if la[r % 2] is None else la[r % 2] + es
                        PP[i][h + z0, pl.ds(r * 16, 16), :] = e.astype(bf16)
                    emarks.append(la[0] + la[1])
                st["l"][(i, h)] = jnp.sum(la[0] + la[1], axis=0, keepdims=True)

        def finish(i, h, oT, l):
            o = oT * ((1.0 - gates[h]) / l)
            if has_mem:
                memT = st["mem"]
                num = memT[h * DH:(h + 1) * DH, i * 128:(i + 1) * 128]
                den = memT[128 + h * 8:128 + (h + 1) * 8, i * 128:(i + 1) * 128] + 1e-6
                w = gates[h] / den
                o = o + num * jnp.concatenate([w] * 4, axis=0)
            return o

        def mem(lag):
            anchor(lag, MTB, PQ[par])
            lhs = jnp.concatenate([MTB[g], ZB[g]], axis=0)
            st["mem"] = _dot_nt(lhs, PQ[par][g])
            marks.append(st["mem"][0:8, 0:128])

        def pv(lag, i):
            nk = (i + 1) * 128
            anchor(lag, VT[par], PP[i])
            outs = []
            for h in range(4):
                vt = jnp.concatenate([VT[par][g, j, pl.ds(h * DH, DH), :] for j in range(i + 1)], axis=1)
                oT = _dot(vt, PP[i][h + z1])
                if h == 0:
                    marks.append(oT[0:8])
                outs.append(finish(i, h, oT, st["l"][(i, h)]))
            oT_all = jnp.concatenate(outs, axis=0).astype(bf16)
            OO[par][g, pl.ds(i * 128, 128), :] = oT_all.T

        def upd(lag):
            anchor(lag, VT[par], PK[par])
            vt_all = jnp.concatenate([VT[par][g, j] for j in range(4)], axis=1)
            dm = _dot(vt_all, PK[par][g])
            marks.append(dm[0:8])
            mt = MT[g] + jnp.where(blockdiag, dm, 0.0)
            MT[g] = mt
            MTB[g] = mt.astype(bf16)
            z = ZZ[g] + jnp.sum(ZC[par][g], axis=0, keepdims=True)
            ZZ[g] = z
            ZB[g] = jnp.concatenate(
                [jnp.where((lane8 >= h * DH) & (lane8 < (h + 1) * DH), z, 0.0) for h in range(4)], axis=0).astype(bf16)

        def fl0(lag, c):
            if c == 0:
                x0_copy(0).wait()
                start_rest()
            rows = pl.ds(c * CH, CH)
            xs = [X0[rows, n * 128:(n + 1) * 128].astype(f32) for n in range(NG)]
            for n in range(NG):
                X[0][n, rows, :] = xs[n]
            ys = _ln_tiles(xs)
            for n in range(NG):
                XN[0][n, rows, :] = ys[n].astype(bf16)

        def w_wait(lag, i):
            w = (WQ, WK, WV)[i]
            pltpu.make_async_copy(w.at[g], w.at[g], sem_w.at[i, g]).wait()

        def fln(lag, t, c):
            first_ln(t, _al((g - 2 * t) * 256 + c * 64, 64), 64)

        table = {"x": lambda lag, c: x0_copy(c).wait(), "g": fl0, "w": w_wait, "lp": o_lp, "f": fln, "qk": qk, "sm": sm, "pv": pv, "mem": mem, "upd": upd,
                 "o": o_proj, "ln": o_ln, "q": q_proj, "k": k_proj, "v": v_proj}
        for kind, args, lag in order:
            table[kind](lag, *args)

    def parse(txt):
        out = []
        for w in txt.split():
            lag = LAG
            if "@" in w:
                w, lg = w.split("@")
                lag = int(lg)
            p = w.split(".")
            out.append((p[0], tuple(int(x) for x in p[1:]), lag))
        names = [t[0] for t in out]
        if "mem" in names and "upd" in names:
            assert names.index("mem") < names.index("upd")
        if "ln" in names:
            assert max(i for i, n in enumerate(names) if n == "o") < names.index("ln")
        return out

    FULL = parse(ORD_FULL)
    FIRST = parse(ORD_FIRST)
    LAST = parse(ORD_LAST)
    PRO = parse(ORD_PRO)
    EPI = parse(ORD_EPI)
    EPI2 = parse(ORD_EPI2)

    body(-1, 0, parse(ORD_START))

    for t in range(NSEG):
        if t > 0:
          for n in range(NG):
              x_copy(t, n).wait()

        if t == 2:
            for n in range(NG):
                w_copy(wo_hbm, WO, 3, n).start()

        def pro0(g, c, t=t):
            for i, w in ((2, WV), (1, WK), (0, WQ)):
                pltpu.make_async_copy(w.at[g], w.at[g], sem_w.at[i, g]).wait()
            body(-1, g, PRO if t == 0 else parse(ORD_PRO0.replace("T", str(t))))
            return c
        lax.fori_loop(max(2 * t, 1), 2 * t + 2, pro0, 0)

    for n in range(NG):
        w_copy(wo_hbm, WO, 3, n).wait()

    def layer(li, carry):
        MT[...] = jnp.zeros(MT.shape, f32)
        ZZ[...] = jnp.zeros(ZZ.shape, f32)
        TOP[0] = jnp.full((8, 128), -jnp.inf, f32)
        TOP[1] = jnp.zeros((8, 128), f32)
        TOP[2] = jnp.full((8, 128), -jnp.inf, f32)
        TOP[3] = jnp.zeros((8, 128), f32)
        def out_copy(s, n):
            return pltpu.make_async_copy(
                XIO[s].at[n], out_hbm.at[pl.ds(s * L, L), pl.ds(n * 128, 128)], sem_o.at[0])

        def loop(s, order, has_mem, extra=None):
            def b(g, c):
                if extra is not None:
                    extra(g)
                body(s, g, order, has_mem)
                return c
            lax.fori_loop(0, NG, b, 0)

        def start_late(g):
            for cp in late_copies(g):
                cp.start()

        def flush(s):
            @pl.when(li == 1)
            def _():
                for n in range(NG):
                    out_copy(s, n).start()

        loop(0, FIRST, False, start_late)
        loop(1, FULL, True)
        loop(2, FULL, True)
        flush(0)
        body(3, 0, LAST, True)

        def b3(g, c):
            body(3, g, LAST, True, (2, g - 1))
            return c
        lax.fori_loop(1, NG, b3, 0)
        flush(1)
        for c in range(NG + 1):
            body(4, c, EPI if c < NG else EPI2, False, (2, NG - 1) if c == 0 else (3, c - 1))
        flush(2)
        flush(3)
        m1, i1, m2, i2 = TOP[0], TOP[1], TOP[2], TOP[3]
        big = f32(1e9)
        ra = jnp.max(m1, axis=0, keepdims=True)
        ia = jnp.min(jnp.where(m1 == ra, i1, big), axis=0, keepdims=True)
        isa = i1 == ia
        cv = jnp.where(isa, m2, m1)
        ci = jnp.where(isa, i2, i1)
        rb = jnp.max(cv, axis=0, keepdims=True)
        ib = jnp.min(jnp.where(cv == rb, ci, big), axis=0, keepdims=True)
        idx = [ia.astype(i32)[0, 0], ib.astype(i32)[0, 0]]
        idx = [jnp.clip(t, 0, S - 1) for t in idx]
        row16 = lax.broadcasted_iota(i32, (16, 128), 0)
        gsel = jnp.where(row16 == 0, jax.nn.sigmoid(ra), jnp.where(row16 == 1, jax.nn.sigmoid(rb), 0.0))

        seg = [t // L for t in idx]
        loc = [t % L for t in idx]
        base = [pl.multiple_of((t // 16) * 16, 16) for t in loc]
        off = [t % 16 for t in loc]
        for t in range(2):
            for s in range(NSEG):
                @pl.when(seg[t] == s)
                def _(t=t, s=s):
                    for n in range(NG):
                        blk = XB[s][n, pl.ds(base[t], 16), :].astype(f32)
                        SEL[t, n] = jnp.broadcast_to(
                            jnp.sum(jnp.where(row16 == off[t], blk, 0.0), axis=0, keepdims=True), (8, 128))
        xsel = []
        for n in range(NG):
            r0_ = SEL[0, n][0:1]
            r1_ = SEL[1, n][0:1]
            xsel.append(jnp.where(row16 == 0, r0_, jnp.where(row16 == 1, r1_, 0.0)))
        xsel = jnp.concatenate(xsel, axis=1).astype(bf16)
        pltpu.make_async_copy(WG, WG, sem_f.at[0]).wait()
        pltpu.make_async_copy(WU, WU, sem_f.at[1]).wait()
        pltpu.make_async_copy(WD, WD, sem_f.at[2]).wait()

        wg = jnp.concatenate([WG[n] for n in range(NF)], axis=1)
        wu = jnp.concatenate([WU[n] for n in range(NF)], axis=1)
        gg = _dot(xsel, wg)
        uu = _dot(xsel, wu)
        hh = (gg * jax.nn.sigmoid(gg) * uu).astype(bf16)
        wd = jnp.concatenate([WD[n] for n in range(NG)], axis=1)
        y = _dot(hh, wd)
        @pl.when(li == 1)
        def _():
            for s in range(NSEG):
                for n in range(NG):
                    out_copy(s, n).wait()

        for t in range(2):
            b8 = pl.multiple_of((loc[t] // 8) * 8, 8)
            o8 = loc[t] % 8
            yrows = []
            for n in range(NG):
                yt = y[:, n * 128:(n + 1) * 128] * gsel
                yrows.append(jnp.sum(jnp.where(row16 == t, yt, 0.0), axis=0, keepdims=True))
            for s in range(NSEG):
                @pl.when(seg[t] == s)
                def _(t=t, s=s, b8=b8, o8=o8, yrows=yrows):
                    xs = []
                    for n in range(NG):
                        blk = X[s][n, pl.ds(b8, 8), :]
                        blk = jnp.where(sub8 == o8, blk + yrows[n], blk)
                        X[s][n, pl.ds(b8, 8), :] = blk
                        xs.append(blk)
                    xn = _ln_tiles(xs)
                    sel = row16 == off[t]
                    for n in range(NG):
                        new_x = jnp.sum(jnp.where(sub8 == o8, xs[n], 0.0), axis=0, keepdims=True)
                        new_n = jnp.sum(jnp.where(sub8 == o8, xn[n], 0.0), axis=0, keepdims=True)
                        blk = XN[s][n, pl.ds(base[t], 16), :]
                        XN[s][n, pl.ds(base[t], 16), :] = jnp.where(sel, new_n, blk.astype(f32)).astype(bf16)
                        blk = XIO[s][n, pl.ds(base[t], 16), :]
                        XIO[s][n, pl.ds(base[t], 16), :] = jnp.where(sel, new_x, blk.astype(f32)).astype(bf16)

                    @pl.when(li == 1)
                    def _():
                        cps = [pltpu.make_async_copy(
                            XIO[s].at[n, pl.ds(base[t], 16), :],
                            out_hbm.at[pl.ds(s * L + base[t], 16), pl.ds(n * 128, 128)], sem_p.at[0])
                            for n in range(NG)]
                        for cp in cps:
                            cp.start()
                        for cp in cps:
                            cp.wait()

        @pl.when(li == 0)
        def _():
            def pro(g, c):
                body(-1, g, PRO)
                return c
            lax.fori_loop(0, NG, pro, 0)
        return carry

    lax.fori_loop(0, 2, layer, 0)


def _build(interpret=False):
    any_spec = pl.BlockSpec(memory_space=pl.ANY)
    vmem_spec = pl.BlockSpec(memory_space=pltpu.VMEM)
    V = pltpu.VMEM
    A = NG + 1
    scratch = (
        [V((NG, L, 128), bf16)] * NSEG + [V((A, L, 128), f32)] * NSEG
        + [V((A, L, 128), bf16)] * NSEG + [V((NG, L, 128), bf16)] * NSEG
        + [V((A, L, 128), bf16)] * 8
        + [V((A, 4, 128, 128), bf16)] * 2
        + [V((A, L, 128), bf16)] * 2
        + [V((NG, 8, 128), f32)] * 2
        + [V((2, (i + 1) * 128, 128), f32) for i in range(4) for _ in range(4)]
        + [V((5, (i + 1) * 128, 128), bf16) for i in range(4)]
    ) + [
        V((A, D, 128), bf16), V((A, D, 128), bf16), V((A, D, 128), bf16), V((A, D, 128), bf16),
        V((NF, D, 128), bf16), V((NF, D, 128), bf16), V((NG, F, 128), bf16),
        V((NG, 128, 128), f32), V((A, 128, 128), bf16),
        V((NG, 8, 128), f32), V((NG, 32, 128), bf16),
        pltpu.SMEM((H,), f32),
        pltpu.SMEM((2,), i32),
        V((4, 8, 128), f32),
        V((2, NG, 8, 128), f32),
        V((NG, 8, 128), f32),
        V((L, D), bf16),
        pltpu.SemaphoreType.DMA((4,)),
        pltpu.SemaphoreType.DMA((NSEG,)),
        pltpu.SemaphoreType.DMA((4, NG)),
        pltpu.SemaphoreType.DMA((3,)),
        pltpu.SemaphoreType.DMA((1,)),
        pltpu.SemaphoreType.DMA((1,)),
    ]
    return pl.pallas_call(
        _kernel,
        out_shape=jax.ShapeDtypeStruct((S, D), bf16),
        in_specs=[any_spec] * 5 + [vmem_spec, vmem_spec] + [any_spec] * 3,
        out_specs=any_spec,
        scratch_shapes=scratch,
        compiler_params=pltpu.CompilerParams(vmem_limit_bytes=110 * 1024 * 1024),
        interpret=pltpu.InterpretParams() if interpret else False,
        name="infini_mod",
    )


@jax.jit
def pallas_interleave_layers__memory_aug_infini_attn__moe_arch_mod__prompt_kernel(
    A_x, A_wq, A_wk, A_wv, A_wo, A_beta, B_x, B_w_r, B_w_gate, B_w_up, B_w_down,
):
    del B_x
    out = _build()(A_x.reshape(S, D), A_wq, A_wk, A_wv, A_wo, A_beta.reshape(1, H), B_w_r.reshape(NG, 128),
                   B_w_gate, B_w_up, B_w_down)
    return out.reshape(1, S, D)
```

```python
import jax
import jax.numpy as jnp
from jax import lax
import jax.experimental.pallas as pl
import jax.experimental.pallas.tpu as pltpu

S = 2048
D = 1024
NSEG = 4
L = S // NSEG
H = 32
DH = D // H
NG = 8
F = 3584
NF = F // 128
CH = L // NG
EPS = 1e-5
LOG2E = 1.4426950408889634
QSCALE = (DH ** -0.5) * LOG2E
NEG = -1e30

ORD_FULL = "o.0.8@0 qk.3@3 qk.0@0 ln.0.1@3 k.0.4 ln.1.1@1 qk.2@0 sm.3.2.2@0 ln.2.2@0 mem@2 qk.1@2 sm.3.0.2@2 v.0.4 pv.3@0 sm.2.2.2@2 sm.2.0.1@2 sm.2.1.1@2 sm.1.0.4@0 pv.2 sm.0.0.4@1 pv.1@2 pv.0@3 q.0.4@0 upd"
ORD_FIRST = "qk.2@2 k.0.4@0 qk.1@3 sm.2.1.3@0 sm.1.0.1@0 v.0.1@0 sm.2.0.1@3 sm.1.1.1@0 qk.3@2 sm.1.2.2@0 q.0.2@0 sm.3.0.4@1 upd@0 qk.0@2 v.3.1@0 sm.0.2.2@3 v.2.1@0 sm.0.0.2@0 v.1.1@3 pv.3@0 pv.0@3 pv.2@3 pv.1@0 q.2.2@0"
ORD_LAST = "qk.2@2 qk.3@2 sm.2.0.1@2 sm.2.2.2@2 sm.2.1.1@2 qk.1@1 sm.3.0.4@2 lp.0.4@3 sm.1.1.1@0 mem@0 sm.1.0.1@3 o.0.4@0 sm.1.3.1@0 qk.0@2 sm.1.2.1@0 pv.2 sm.0.0.4@0 pv.3@3 pv.1@0 pv.0@2 o.4.4@0"
ORD_START = "g.0 g.1 x.1 x.2 x.3 w.2 w.0 w.1 v.0.1@0 g.2 g.3 v.1.1@0 g.4 g.5 v.2.1@0 g.6 g.7 v.3.1@0 q.0.4@0 k.0.1@0 k.1.1@0 k.2.2@0"
ORD_PRO = "v.0.4 q.0.4@0 k.0.1@0 k.1.1@0 k.2.2@0"
ORD_EPI = "lp.1.1@0 lp.2.2@0 lp.0.1@1 o.0.8@0"
ORD_EPI2 = "lp.0.4@0"
ORD_PRO0 = "v.0.4 f.T.0 f.T.1 q.0.4@0 f.T.2 f.T.3 k.0.1@0 k.1.1@0 k.2.2@0"
LAG = 2
EL = 3

bf16 = jnp.bfloat16
f32 = jnp.float32
u32 = jnp.uint32
i32 = jnp.int32
NT = (((1,), (1,)), ((), ()))


def _al(i, m):
    return i if isinstance(i, int) else pl.multiple_of(i, m)


def _dot(a, b):
    return jnp.dot(a, b, preferred_element_type=f32)


def _dot_nt(a, b):
    return lax.dot_general(a, b, NT, preferred_element_type=f32)


def _phi(t):
    return jnp.where(t > 0, t + 1.0, jnp.exp(t))


def _ln_tiles(xs):
    tot = xs[0]
    for x in xs[1:]:
        tot = tot + x
    mean = jnp.sum(tot, axis=-1, keepdims=True) * (1.0 / D)
    ds = [x - mean for x in xs]
    sq = ds[0] * ds[0]
    for d in ds[1:]:
        sq = sq + d * d
    var = jnp.sum(sq, axis=-1, keepdims=True) * (1.0 / D)
    rstd = lax.rsqrt(var + EPS)
    return [d * rstd for d in ds]


def _kernel(x_hbm, wq_hbm, wk_hbm, wv_hbm, wo_hbm, beta_ref, wr_ref, wg_hbm, wu_hbm, wd_hbm,
            out_hbm, *scr):
    scr = list(scr)

    def take(n):
        out = scr[:n]
        del scr[:n]
        return out
    XIO, X, XN, XB = take(NSEG), take(NSEG), take(NSEG), take(NSEG)
    QS, PQ, KK, PK, VT, OO, ZC = take(2), take(2), take(2), take(2), take(2), take(2), take(2)
    SS = [take(4) for _ in range(4)]
    PP = take(4)
    (WQ, WK, WV, WO, WG, WU, WD, MT, MTB, ZZ, ZB, GATE, ZO, TOP, SEL, WR, X0,
     sem_0, sem_x, sem_w, sem_f, sem_o, sem_p) = scr

    def x_copy(s, n):
        return pltpu.make_async_copy(
            x_hbm.at[pl.ds(s * L, L), pl.ds(n * 128, 128)], XIO[s].at[n], sem_x.at[s])

    def w_copy(w_hbm, buf, i, n):
        return pltpu.make_async_copy(w_hbm.at[:, pl.ds(_al(n * 128, 128), 128)], buf.at[n], sem_w.at[i, n])

    def f_copy(w_hbm, buf, i, n):
        return pltpu.make_async_copy(w_hbm.at[:, pl.ds(_al(n * 128, 128), 128)], buf.at[n], sem_f.at[i])
    def start_w(n):
        w_copy(wv_hbm, WV, 2, n).start()
        w_copy(wk_hbm, WK, 1, n).start()
        w_copy(wq_hbm, WQ, 0, n).start()

    def x0_copy(c):
        rows = pl.ds(c * 128, 128)
        return pltpu.make_async_copy(x_hbm.at[rows, :], X0.at[rows, :], sem_0.at[c])

    for c in range(4):
        x0_copy(c).start()
    start_w(0)

    def start_rest():
        start_w(1)
        for s in range(1, NSEG):
            for n in range(NG):
                x_copy(s, n).start()
            start_w(2 * s)
            start_w(2 * s + 1)
    def late_copies(g):
        cps = [f_copy(wd_hbm, WD, 2, g)]
        for w_hbm, buf, i in ((wg_hbm, WG, 0), (wu_hbm, WU, 1)):
            for t in range(3):
                cps.append(f_copy(w_hbm, buf, i, g + NG * t))
            r0 = _al((g % 2) * (D // 2), D // 2)
            n = 3 * NG + g // 2
            cps.append(pltpu.make_async_copy(
                w_hbm.at[pl.ds(r0, D // 2), pl.ds(_al(n * 128, 128), 128)],
                buf.at[n, pl.ds(r0, D // 2), :], sem_f.at[i]))
        return cps

    lane = lax.broadcasted_iota(i32, (128, 128), 1)
    row = lax.broadcasted_iota(i32, (128, 128), 0)
    causal = row <= lane
    blockdiag = (row // DH) == (lane // DH)
    lane64 = lax.broadcasted_iota(i32, (64, 128), 1)
    hmask = [jnp.where((lane64 >= h * DH) & (lane64 < (h + 1) * DH), u32(0xFFFFFFFF), u32(0)) for h in range(4)]
    lane8 = lax.broadcasted_iota(i32, (8, 128), 1)
    sub8 = lax.broadcasted_iota(i32, (8, 128), 0)
    ZO[0] = 0
    ZO[1] = 0
    gv = jax.nn.sigmoid(beta_ref[...].astype(f32))
    for h in range(H):
        GATE[h] = gv[0, h]

    for n in range(NG):
        WR[n] = jnp.broadcast_to(wr_ref[n:n + 1, :].astype(f32), (8, 128))
    def first_ln(t, r0, rows):
        xs = [XIO[t][n, pl.ds(r0, rows), :].astype(f32) for n in range(NG)]
        for n in range(NG):
            X[t][n, pl.ds(r0, rows), :] = xs[n]
        ys = _ln_tiles(xs)
        for n in range(NG):
            XN[t][n, pl.ds(r0, rows), :] = ys[n].astype(bf16)

    def body(s, g, order, has_mem=False, prev=None):
        par = s % 2
        z0, z1 = ZO[0], ZO[1]
        marks = []
        emarks = []
        st = {"m": {}, "mx": {}, "l": {}, "mem": None, "zc": None}
        gates = [GATE[g * 4 + h] for h in range(4)]

        def anchor(lag, *refs):
            lag = min(lag, len(marks))
            if lag == 0:
                return
            mk = marks[-lag]
            for ref in refs:
                slot = ref.shape[0] - 1
                if ref.dtype == f32:
                    val = mk
                else:
                    val = jnp.concatenate([mk, mk], axis=0).astype(ref.dtype)
                idx = (slot + z0,) + (0,) * (len(ref.shape) - 3) + (pl.ds(_al(z0 * val.shape[0], val.shape[0]), val.shape[0]), slice(None))
                ref[idx] = val

        def xn_lhs(t, c, nc):
            return jnp.concatenate([XN[t][k, pl.ds(c * 128, nc * 128), :] for k in range(NG)], axis=1)

        def q_proj(lag, c, nc=1):
            t, tp = s + 1, 1 - par
            anchor(lag, XN[t], WQ)
            q = _dot(xn_lhs(t, c, nc), WQ[g])
            marks.append(q[0:8])
            rows = pl.ds(c * 128, nc * 128)
            QS[tp][g, rows, :] = (q * QSCALE).astype(bf16)
            PQ[tp][g, rows, :] = _phi(q).astype(bf16)

        def k_proj(lag, c, nc=1):
            t, tp = s + 1, 1 - par
            anchor(lag, XN[t], WK)
            k = _dot(xn_lhs(t, c, nc), WK[g])
            marks.append(k[0:8])
            rows = pl.ds(c * 128, nc * 128)
            KK[tp][g, rows, :] = k.astype(bf16)
            pk = _phi(k)
            PK[tp][g, rows, :] = pk.astype(bf16)
            zc = st["zc"]
            for r in range(nc * 16):
                zc = pk[r * 8:(r + 1) * 8] if zc is None else zc + pk[r * 8:(r + 1) * 8]
            st["zc"] = zc
            if c + nc == 4:
                ZC[tp][g] = zc

        def v_proj(lag, c, nc=1):
            t, tp = s + 1, 1 - par
            anchor(lag, XN[t], WV)
            v = _dot(xn_lhs(t, c, nc), WV[g])
            marks.append(v[0:8])
            v = v.astype(bf16)
            for j in range(nc):
                VT[tp][g, c + j] = v[j * 128:(j + 1) * 128, :].T

        def o_proj(lag, n0, nn=2):
            t, tp = s - 1, 1 - par
            cr = _al(g * CH, CH)
            anchor(lag, OO[tp], WO)
            lhs = jnp.concatenate([OO[tp][k, pl.ds(cr, CH), :] for k in range(NG)], axis=1)
            rhs = jnp.concatenate([WO[n] for n in range(n0, n0 + nn)], axis=1)
            att = _dot(lhs, rhs)
            marks.append(att[0:8, 0:128])
            for i in range(nn):
                n = n0 + i
                X[t][n + z0, pl.ds(cr, CH), :] = X[t][n, pl.ds(cr, CH), :] + att[:, i * 128:(i + 1) * 128]

        def o_lp(lag, c, nc=1):
            if prev is not None:
                o_ln(lag, c, nc, *prev)

        def o_ln(lag, c, nc=1, t=s - 1, g=g):
            anchor(lag, X[t])
            R = 16 * nc
            r0 = _al(g * CH + c * 16, 16)
            x1 = [X[t][n + z1, pl.ds(r0, R), :] for n in range(NG)]
            xb = _ln_tiles(x1)
            wr = [jnp.concatenate([WR[n]] * (R // 8), axis=0) for n in range(NG)]
            acc = xb[0] * wr[0]
            for n in range(1, NG):
                acc = acc + xb[n] * wr[n]
            r = jnp.broadcast_to(jnp.sum(acc, axis=-1, keepdims=True), (R, 128))
            m1, i1, m2, i2 = TOP[0], TOP[1], TOP[2], TOP[3]
            for u in range(R // 8):
                rv = r[u * 8:(u + 1) * 8, :]
                iv = (sub8 + (r0 + (t * L + u * 8))).astype(f32)
                g1 = rv > m1
                g2 = rv > m2
                m2 = jnp.where(g1, m1, jnp.where(g2, rv, m2))
                i2 = jnp.where(g1, i1, jnp.where(g2, iv, i2))
                m1 = jnp.where(g1, rv, m1)
                i1 = jnp.where(g1, iv, i1)
            TOP[0] = m1
            TOP[1] = i1
            TOP[2] = m2
            TOP[3] = i2
            x2 = [x1[n] + xb[n] for n in range(NG)]
            for n in range(NG):
                X[t][n, pl.ds(r0, R), :] = x2[n]
                XB[t][n, pl.ds(r0, R), :] = xb[n].astype(bf16)
                XIO[t][n, pl.ds(r0, R), :] = x2[n].astype(bf16)
            xn = _ln_tiles(x2)
            for n in range(NG):
                XN[t][n, pl.ds(r0, R), :] = xn[n].astype(bf16)

        def qk(lag, i):
            nk = (i + 1) * 128
            anchor(lag, QS[par], KK[par])
            qu = pltpu.bitcast(QS[par][g, pl.ds(i * 128, 128), :], u32)
            qm = jnp.concatenate([pltpu.bitcast(qu & hmask[h], bf16) for h in range(4)], axis=0)
            sT = _dot_nt(KK[par][g, pl.ds(0, nk), :], qm)
            marks.append(sT[0:8, 0:128])
            for h in range(4):
                mx = None
                for r in range(nk // 8):
                    t = sT[r * 8:(r + 1) * 8, h * 128:(h + 1) * 128]
                    if r >= i * 16:
                        t = jnp.where(causal[(r - i * 16) * 8:(r - i * 16 + 1) * 8], t, NEG)
                    mx = t if mx is None else jnp.maximum(mx, t)
                    SS[i][h][z0, pl.ds(r * 8, 8), :] = t
                st["m"][(i, h)] = jnp.max(mx, axis=0, keepdims=True)

        def sm(lag, i, h0, nh=1):
            for h in range(h0, h0 + nh):
                m = st["m"][(i, h)]
                la = [None, None]
                for j in range(i + 1):
                    if len(emarks) >= EL:
                        SS[i][h][1 + z0, pl.ds(_al(z0 * 8, 8), 8), :] = emarks[-EL]
                    else:
                        anchor(lag, SS[i][h])
                    for r in range(j * 8, (j + 1) * 8):
                        e = jnp.exp2(SS[i][h][z1, pl.ds(r * 16, 16), :] - m)
                        es = e[0:8] + e[8:16]
                        la[r % 2] = es if la[r % 2] is None else la[r % 2] + es
                        PP[i][h + z0, pl.ds(r * 16, 16), :] = e.astype(bf16)
                    emarks.append(la[0] + la[1])
                st["l"][(i, h)] = jnp.sum(la[0] + la[1], axis=0, keepdims=True)

        def finish(i, h, oT, l):
            o = oT * ((1.0 - gates[h]) / l)
            if has_mem:
                memT = st["mem"]
                num = memT[h * DH:(h + 1) * DH, i * 128:(i + 1) * 128]
                den = memT[128 + h * 8:128 + (h + 1) * 8, i * 128:(i + 1) * 128] + 1e-6
                w = gates[h] / den
                o = o + num * jnp.concatenate([w] * 4, axis=0)
            return o

        def mem(lag):
            anchor(lag, MTB, PQ[par])
            lhs = jnp.concatenate([MTB[g], ZB[g]], axis=0)
            st["mem"] = _dot_nt(lhs, PQ[par][g])
            marks.append(st["mem"][0:8, 0:128])

        def pv(lag, i):
            nk = (i + 1) * 128
            anchor(lag, VT[par], PP[i])
            outs = []
            for h in range(4):
                vt = jnp.concatenate([VT[par][g, j, pl.ds(h * DH, DH), :] for j in range(i + 1)], axis=1)
                oT = _dot(vt, PP[i][h + z1])
                if h == 0:
                    marks.append(oT[0:8])
                outs.append(finish(i, h, oT, st["l"][(i, h)]))
            oT_all = jnp.concatenate(outs, axis=0).astype(bf16)
            OO[par][g, pl.ds(i * 128, 128), :] = oT_all.T

        def upd(lag):
            anchor(lag, VT[par], PK[par])
            vt_all = jnp.concatenate([VT[par][g, j] for j in range(4)], axis=1)
            dm = _dot(vt_all, PK[par][g])
            marks.append(dm[0:8])
            mt = MT[g] + jnp.where(blockdiag, dm, 0.0)
            MT[g] = mt
            MTB[g] = mt.astype(bf16)
            z = ZZ[g] + jnp.sum(ZC[par][g], axis=0, keepdims=True)
            ZZ[g] = z
            ZB[g] = jnp.concatenate(
                [jnp.where((lane8 >= h * DH) & (lane8 < (h + 1) * DH), z, 0.0) for h in range(4)], axis=0).astype(bf16)

        def fl0(lag, c):
            if c == 0:
                x0_copy(0).wait()
                start_rest()
            rows = pl.ds(c * CH, CH)
            xs = [X0[rows, n * 128:(n + 1) * 128].astype(f32) for n in range(NG)]
            for n in range(NG):
                X[0][n, rows, :] = xs[n]
            ys = _ln_tiles(xs)
            for n in range(NG):
                XN[0][n, rows, :] = ys[n].astype(bf16)

        def w_wait(lag, i):
            w = (WQ, WK, WV)[i]
            pltpu.make_async_copy(w.at[g], w.at[g], sem_w.at[i, g]).wait()

        def fln(lag, t, c):
            first_ln(t, _al((g - 2 * t) * 256 + c * 64, 64), 64)

        table = {"x": lambda lag, c: x0_copy(c).wait(), "g": fl0, "w": w_wait, "lp": o_lp, "f": fln, "qk": qk, "sm": sm, "pv": pv, "mem": mem, "upd": upd,
                 "o": o_proj, "ln": o_ln, "q": q_proj, "k": k_proj, "v": v_proj}
        for kind, args, lag in order:
            table[kind](lag, *args)

    def parse(txt):
        out = []
        for w in txt.split():
            lag = LAG
            if "@" in w:
                w, lg = w.split("@")
                lag = int(lg)
            p = w.split(".")
            out.append((p[0], tuple(int(x) for x in p[1:]), lag))
        names = [t[0] for t in out]
        if "mem" in names and "upd" in names:
            assert names.index("mem") < names.index("upd")
        if "ln" in names:
            assert max(i for i, n in enumerate(names) if n == "o") < names.index("ln")
        return out

    FULL = parse(ORD_FULL)
    FIRST = parse(ORD_FIRST)
    LAST = parse(ORD_LAST)
    PRO = parse(ORD_PRO)
    EPI = parse(ORD_EPI)
    EPI2 = parse(ORD_EPI2)

    body(-1, 0, parse(ORD_START))

    for t in range(NSEG):
        if t > 0:
          for n in range(NG):
              x_copy(t, n).wait()

        if t == 2:
            for n in range(NG):
                w_copy(wo_hbm, WO, 3, n).start()

        def pro0(g, c, t=t):
            for i, w in ((2, WV), (1, WK), (0, WQ)):
                pltpu.make_async_copy(w.at[g], w.at[g], sem_w.at[i, g]).wait()
            body(-1, g, PRO if t == 0 else parse(ORD_PRO0.replace("T", str(t))))
            return c
        lax.fori_loop(max(2 * t, 1), 2 * t + 2, pro0, 0)

    for n in range(NG):
        w_copy(wo_hbm, WO, 3, n).wait()

    def layer(li, carry):
        MT[...] = jnp.zeros(MT.shape, f32)
        ZZ[...] = jnp.zeros(ZZ.shape, f32)
        TOP[0] = jnp.full((8, 128), -jnp.inf, f32)
        TOP[1] = jnp.zeros((8, 128), f32)
        TOP[2] = jnp.full((8, 128), -jnp.inf, f32)
        TOP[3] = jnp.zeros((8, 128), f32)
        def out_copy(s, n):
            return pltpu.make_async_copy(
                XIO[s].at[n], out_hbm.at[pl.ds(s * L, L), pl.ds(n * 128, 128)], sem_o.at[0])

        def loop(s, order, has_mem, extra=None):
            def b(g, c):
                if extra is not None:
                    extra(g)
                body(s, g, order, has_mem)
                return c
            lax.fori_loop(0, NG, b, 0)

        def start_late(g):
            for cp in late_copies(g):
                cp.start()

        def flush(s):
            @pl.when(li == 1)
            def _():
                for n in range(NG):
                    out_copy(s, n).start()

        loop(0, FIRST, False, start_late)
        loop(1, FULL, True)
        loop(2, FULL, True)
        flush(0)
        body(3, 0, LAST, True)

        def b3(g, c):
            body(3, g, LAST, True, (2, g - 1))
            return c
        lax.fori_loop(1, NG, b3, 0)
        flush(1)
        body(4, 0, EPI, False, (2, NG - 1))

        def epi(c, carry):
            body(4, c, EPI, False, (3, c - 1))
            return carry
        lax.fori_loop(1, NG, epi, 0)
        body(4, NG, EPI2, False, (3, NG - 1))
        flush(2)
        flush(3)
        m1, i1, m2, i2 = TOP[0], TOP[1], TOP[2], TOP[3]
        big = f32(1e9)
        ra = jnp.max(m1, axis=0, keepdims=True)
        ia = jnp.min(jnp.where(m1 == ra, i1, big), axis=0, keepdims=True)
        isa = i1 == ia
        cv = jnp.where(isa, m2, m1)
        ci = jnp.where(isa, i2, i1)
        rb = jnp.max(cv, axis=0, keepdims=True)
        ib = jnp.min(jnp.where(cv == rb, ci, big), axis=0, keepdims=True)
        idx = [ia.astype(i32)[0, 0], ib.astype(i32)[0, 0]]
        idx = [jnp.clip(t, 0, S - 1) for t in idx]
        row16 = lax.broadcasted_iota(i32, (16, 128), 0)
        gsel = jnp.where(row16 == 0, jax.nn.sigmoid(ra), jnp.where(row16 == 1, jax.nn.sigmoid(rb), 0.0))

        seg = [t // L for t in idx]
        loc = [t % L for t in idx]
        base = [pl.multiple_of((t // 16) * 16, 16) for t in loc]
        off = [t % 16 for t in loc]
        for t in range(2):
            for s in range(NSEG):
                @pl.when(seg[t] == s)
                def _(t=t, s=s):
                    for n in range(NG):
                        blk = XB[s][n, pl.ds(base[t], 16), :].astype(f32)
                        SEL[t, n] = jnp.broadcast_to(
                            jnp.sum(jnp.where(row16 == off[t], blk, 0.0), axis=0, keepdims=True), (8, 128))
        xsel = []
        for n in range(NG):
            r0_ = SEL[0, n][0:1]
            r1_ = SEL[1, n][0:1]
            xsel.append(jnp.where(row16 == 0, r0_, jnp.where(row16 == 1, r1_, 0.0)))
        xsel = jnp.concatenate(xsel, axis=1).astype(bf16)
        pltpu.make_async_copy(WG, WG, sem_f.at[0]).wait()
        pltpu.make_async_copy(WU, WU, sem_f.at[1]).wait()
        pltpu.make_async_copy(WD, WD, sem_f.at[2]).wait()

        wg = jnp.concatenate([WG[n] for n in range(NF)], axis=1)
        wu = jnp.concatenate([WU[n] for n in range(NF)], axis=1)
        gg = _dot(xsel, wg)
        uu = _dot(xsel, wu)
        hh = (gg * jax.nn.sigmoid(gg) * uu).astype(bf16)
        wd = jnp.concatenate([WD[n] for n in range(NG)], axis=1)
        y = _dot(hh, wd)
        @pl.when(li == 1)
        def _():
            for s in range(NSEG):
                for n in range(NG):
                    out_copy(s, n).wait()

        for t in range(2):
            b8 = pl.multiple_of((loc[t] // 8) * 8, 8)
            o8 = loc[t] % 8
            yrows = []
            for n in range(NG):
                yt = y[:, n * 128:(n + 1) * 128] * gsel
                yrows.append(jnp.sum(jnp.where(row16 == t, yt, 0.0), axis=0, keepdims=True))
            for s in range(NSEG):
                @pl.when(seg[t] == s)
                def _(t=t, s=s, b8=b8, o8=o8, yrows=yrows):
                    xs = []
                    for n in range(NG):
                        blk = X[s][n, pl.ds(b8, 8), :]
                        blk = jnp.where(sub8 == o8, blk + yrows[n], blk)
                        X[s][n, pl.ds(b8, 8), :] = blk
                        xs.append(blk)
                    xn = _ln_tiles(xs)
                    sel = row16 == off[t]
                    for n in range(NG):
                        new_x = jnp.sum(jnp.where(sub8 == o8, xs[n], 0.0), axis=0, keepdims=True)
                        new_n = jnp.sum(jnp.where(sub8 == o8, xn[n], 0.0), axis=0, keepdims=True)
                        blk = XN[s][n, pl.ds(base[t], 16), :]
                        XN[s][n, pl.ds(base[t], 16), :] = jnp.where(sel, new_n, blk.astype(f32)).astype(bf16)
                        blk = XIO[s][n, pl.ds(base[t], 16), :]
                        XIO[s][n, pl.ds(base[t], 16), :] = jnp.where(sel, new_x, blk.astype(f32)).astype(bf16)

                    @pl.when(li == 1)
                    def _():
                        cps = [pltpu.make_async_copy(
                            XIO[s].at[n, pl.ds(base[t], 16), :],
                            out_hbm.at[pl.ds(s * L + base[t], 16), pl.ds(n * 128, 128)], sem_p.at[0])
                            for n in range(NG)]
                        for cp in cps:
                            cp.start()
                        for cp in cps:
                            cp.wait()

        @pl.when(li == 0)
        def _():
            def pro(g, c):
                body(-1, g, PRO)
                return c
            lax.fori_loop(0, NG, pro, 0)
        return carry

    lax.fori_loop(0, 2, layer, 0)


def _build(interpret=False):
    any_spec = pl.BlockSpec(memory_space=pl.ANY)
    vmem_spec = pl.BlockSpec(memory_space=pltpu.VMEM)
    V = pltpu.VMEM
    A = NG + 1
    scratch = (
        [V((NG, L, 128), bf16)] * NSEG + [V((A, L, 128), f32)] * NSEG
        + [V((A, L, 128), bf16)] * NSEG + [V((NG, L, 128), bf16)] * NSEG
        + [V((A, L, 128), bf16)] * 8
        + [V((A, 4, 128, 128), bf16)] * 2
        + [V((A, L, 128), bf16)] * 2
        + [V((NG, 8, 128), f32)] * 2
        + [V((2, (i + 1) * 128, 128), f32) for i in range(4) for _ in range(4)]
        + [V((5, (i + 1) * 128, 128), bf16) for i in range(4)]
    ) + [
        V((A, D, 128), bf16), V((A, D, 128), bf16), V((A, D, 128), bf16), V((A, D, 128), bf16),
        V((NF, D, 128), bf16), V((NF, D, 128), bf16), V((NG, F, 128), bf16),
        V((NG, 128, 128), f32), V((A, 128, 128), bf16),
        V((NG, 8, 128), f32), V((NG, 32, 128), bf16),
        pltpu.SMEM((H,), f32),
        pltpu.SMEM((2,), i32),
        V((4, 8, 128), f32),
        V((2, NG, 8, 128), f32),
        V((NG, 8, 128), f32),
        V((L, D), bf16),
        pltpu.SemaphoreType.DMA((4,)),
        pltpu.SemaphoreType.DMA((NSEG,)),
        pltpu.SemaphoreType.DMA((4, NG)),
        pltpu.SemaphoreType.DMA((3,)),
        pltpu.SemaphoreType.DMA((1,)),
        pltpu.SemaphoreType.DMA((1,)),
    ]
    return pl.pallas_call(
        _kernel,
        out_shape=jax.ShapeDtypeStruct((S, D), bf16),
        in_specs=[any_spec] * 5 + [vmem_spec, vmem_spec] + [any_spec] * 3,
        out_specs=any_spec,
        scratch_shapes=scratch,
        compiler_params=pltpu.CompilerParams(vmem_limit_bytes=110 * 1024 * 1024),
        interpret=pltpu.InterpretParams() if interpret else False,
        name="infini_mod",
    )


@jax.jit
def pallas_interleave_layers__memory_aug_infini_attn__moe_arch_mod__prompt_kernel(
    A_x, A_wq, A_wk, A_wv, A_wo, A_beta, B_x, B_w_r, B_w_gate, B_w_up, B_w_down,
):
    del B_x
    out = _build()(A_x.reshape(S, D), A_wq, A_wk, A_wv, A_wo, A_beta.reshape(1, H), B_w_r.reshape(NG, 128),
                   B_w_gate, B_w_up, B_w_down)
    return out.reshape(1, S, D)
```
